```python
import os as _os
_os.environ.setdefault("JAX_PLATFORMS", "cpu")
import jax
import jax.numpy as jnp

def _softmax(x, axis=-1):
    return jax.nn.softmax(x, axis=axis)
def _gelu(x):
    return jax.nn.gelu(x, approximate=True)
def _silu(x):
    return jax.nn.silu(x)
def _sigmoid(x):
    return jax.nn.sigmoid(x)
def _layernorm(x, axis=-1, eps=1e-5):
    m = jnp.mean(x, axis=axis, keepdims=True)
    v = jnp.var(x, axis=axis, keepdims=True)
    return (x - m) / jnp.sqrt(v + eps)
def _scatter_add(tgt, idx, src, axis=0):
    return tgt.at[idx].add(src)
def _segment_sum(src, seg, n):
    return jax.ops.segment_sum(src, seg, n)
class _Rng:
    def __init__(self, key):
        self._k = key
    def _next(self):
        self._k, sub = jax.random.split(self._k)
        return sub
    def normal(self, shape):
        return jax.random.normal(self._next(), shape, dtype=jnp.bfloat16)
    def randint(self, lo, hi, shape):
        return jax.random.randint(self._next(), shape, lo, hi, dtype=jnp.int32)
    def uniform(self, shape, lo=0.0, hi=1.0):
        return jax.random.uniform(self._next(), shape, jnp.bfloat16, lo, hi)
    def permutation(self, n):
        return jax.random.permutation(self._next(), n)


kernel_name = 'sequential_preLN__softmax_full_mha__dense_activation_gelu__prompt'

def setup_inputs():
    _rng = _Rng(jax.random.key(int.from_bytes(__import__("os").urandom(4), "little")))
    _w = (lambda a: (lambda t: t.astype(jnp.bfloat16) if jnp.issubdtype(t.dtype, jnp.floating) else t)(jnp.asarray(a)))
    def _A_setup():
        B, S, D = 1, 2048, 512
        return {
            "x": _w((lambda *s: _rng.normal(s) * 0.05)(B, S, D)),
            "wqkv": _w((lambda *s: _rng.normal(s) * 0.05)(D, 3 * D)),
            "wo": _w((lambda *s: _rng.normal(s) * 0.05)(D, D)),
        }
    _A_in = _A_setup()

    def _B_setup():
        B, S, D, F = 1, 2048, 512, 1792
        return {
            "x": _w((lambda *s: _rng.normal(s) * 0.05)(B, S, D)),
            "w1": _w((lambda *s: _rng.normal(s) * 0.4)(D, F) * (D ** -0.5)),
            "b1": _w((lambda *s: _rng.normal(s) * 0.4)(F) * 0.01),
            "w2": _w((lambda *s: _rng.normal(s) * 0.4)(F, D) * (F ** -0.5)),
            "b2": _w((lambda *s: _rng.normal(s) * 0.05)(D) * 0.01),
        }
    _B_in = _B_setup()

    return {
        "A_x": _A_in["x"],
        "A_wqkv": _A_in["wqkv"],
        "A_wo": _A_in["wo"],
        "B_x": _B_in["x"],
        "B_w1": _B_in["w1"],
        "B_b1": _B_in["b1"],
        "B_w2": _B_in["w2"],
        "B_b2": _B_in["b2"],
    }

def reference(A_x, A_wqkv, A_wo, B_x, B_w1, B_b1, B_w2, B_b2):
    def _A_ref(x, wqkv, wo):
        B, S, D = x.shape
        H = 32; Dh = D // H
        qkv = (lambda x, *d: x.transpose(*d))((x @ wqkv).reshape(B, S, 3, H, Dh), 2, 0, 3, 1, 4)
        q, k, v = qkv[0], qkv[1], qkv[2]
        scale = Dh ** -0.5
        scores = jnp.einsum("bhqd,bhkd->bhqk", q, k) * scale
        p = _softmax(scores, axis=-1)
        o = jnp.einsum("bhqk,bhkd->bhqd", p, v)
        return (lambda x, *d: x.transpose(*d))(o, 0, 2, 1, 3).reshape(B, S, D) @ wo

    def _B_ref(x, w1, b1, w2, b2):
        h = jnp.einsum("bsd,df->bsf", x, w1) + b1
        h = _gelu(h)
        return jnp.einsum("bsf,fd->bsd", h, w2) + b2

    x = A_x
    h = x + _A_ref(_layernorm(x, axis=-1), A_wqkv, A_wo)
    h2 = h + _B_ref(_layernorm(h, axis=-1), B_w1, B_b1, B_w2, B_b2)
    return h2
```

```python
import functools
import math

import jax
import jax.numpy as jnp
import jax.experimental.pallas as pl
import jax.experimental.pallas.tpu as pltpu

F32 = jnp.float32
BF16 = jnp.bfloat16

_H = 32
_EPS = 1e-5
_LOG2E = math.log2(math.e)
_SAFE_LOG2 = 60.0
_SAFE_V = 2.0 ** 40


def _layernorm(x):
    m = jnp.mean(x, axis=-1, keepdims=True)
    xc = x - m
    v = jnp.mean(xc * xc, axis=-1, keepdims=True)
    return xc * jax.lax.rsqrt(v + _EPS)


def _dot(a, b):
    return jnp.dot(a, b, preferred_element_type=F32)


def _dot_nt(a, b):
    return jax.lax.dot_general(a, b, (((1,), (1,)), ((), ())), preferred_element_type=F32)


def _kernel(x_ref, wqkv_ref, wo_ref, w1_ref, b1_ref, w2_ref, b2_ref, o_ref,
            k_scr, qt_scr, vt_scr, ot_scr, flag_ref, *, S, D, BQ, CK, TB):
    H = _H
    Dh = D // H
    HG = 128 // Dh
    NG = H // HG
    NC = S // CK
    i = pl.program_id(0)

    @pl.when(i == 0)
    def _():
        qscale = (Dh ** -0.5) * _LOG2E
        wq_t = wqkv_ref[:, 0:D].T
        wv_t = wqkv_ref[:, 2 * D:3 * D].T
        wk = wqkv_ref[:, D:2 * D]
        qn_max = jnp.zeros((H, TB), F32)
        kk_max = jnp.zeros((TB // 8, D), F32)
        v_max = jnp.zeros((8, TB), F32)
        for tb in range(S // TB):
            rows = slice(tb * TB, (tb + 1) * TB)
            xn = _layernorm(x_ref[rows, :].astype(F32)).astype(BF16)
            k = _dot(xn, wk).astype(BF16)
            for g in range(NG):
                k_scr[g, rows, :] = k[:, g * 128:(g + 1) * 128]
            qt = (_dot_nt(wq_t, xn) * qscale).astype(BF16)
            vt = _dot_nt(wv_t, xn).astype(BF16)
            qt_scr[(tb * TB) // BQ, :, (tb * TB) % BQ:(tb * TB) % BQ + TB] = qt
            vt_scr[:, rows] = vt
            qf = qt.astype(F32)
            qn_max = jnp.maximum(qn_max, jnp.sum((qf * qf).reshape(H, Dh, TB), axis=1))
            kf = k.astype(F32)
            kk_max = jnp.maximum(kk_max, jnp.max((kf * kf).reshape(8, TB // 8, D), axis=0))
            v_max = jnp.maximum(v_max, jnp.max(jnp.abs(vt.astype(F32)).reshape(D // 8, 8, TB), axis=0))
        seg = (jax.lax.broadcasted_iota(jnp.int32, (D, 128), 0) // Dh
               == jax.lax.broadcasted_iota(jnp.int32, (D, 128), 1)).astype(BF16)
        kn = _dot((kk_max * 1.02).astype(BF16), seg)
        bound2 = jnp.max(qn_max) * jnp.max(kn)
        ok = jnp.logical_and(bound2 <= _SAFE_LOG2 * _SAFE_LOG2, jnp.max(v_max) <= _SAFE_V)
        flag_ref[0] = ok.astype(jnp.int32)

    def masked_q(g, hh):
        r0 = pl.multiple_of(g * 128 + hh * Dh, Dh)
        q = qt_scr[i, pl.ds(r0, Dh), :]
        parts = []
        if hh > 0:
            parts.append(jnp.zeros((hh * Dh, BQ), BF16))
        parts.append(q)
        if hh < HG - 1:
            parts.append(jnp.zeros(((HG - 1 - hh) * Dh, BQ), BF16))
        return jnp.concatenate(parts, axis=0)

    def v_rows(g, hh, c):
        r0 = pl.multiple_of(g * 128 + hh * Dh, Dh)
        return vt_scr[pl.ds(r0, Dh), c * CK:(c + 1) * CK]

    def finish(g, hh, acc, lsum):
        r0 = pl.multiple_of(g * 128 + hh * Dh, Dh)
        l = jnp.sum(lsum, axis=0, keepdims=True)
        ot_scr[pl.ds(r0, Dh), :] = acc / l

    fast = flag_ref[0] == 1

    @pl.when(fast)
    def _():
        def group(g, carry):
            seq = [(hh, c) for hh in range(HG) for c in range(NC)]
            n = len(seq)
            wq = {}
            acc = {}
            lsum = {}
            pts = {}

            def qk(j):
                hh, c = seq[j]
                if c == 0:
                    wq[hh] = masked_q(g, hh)
                st = _dot(k_scr[g, c * CK:(c + 1) * CK, :], wq[hh])
                p = jnp.exp2(st)
                ps = jnp.sum(p.reshape(CK // 8, 8, BQ), axis=0)
                lsum[hh] = ps if c == 0 else lsum[hh] + ps
                pts[j] = p.astype(BF16)

            def pv(j):
                hh, c = seq[j]
                o = _dot(v_rows(g, hh, c), pts.pop(j))
                acc[hh] = o if c == 0 else acc[hh] + o
                if c == NC - 1:
                    finish(g, hh, acc.pop(hh), lsum.pop(hh))

            for j in range(n + 1):
                if j < n:
                    qk(j)
                if j >= 1:
                    pv(j - 1)
            return carry
        jax.lax.fori_loop(0, NG, group, 0)

    @pl.when(jnp.logical_not(fast))
    def _():
        def group(g, carry):
            for hh in range(HG):
                wq = masked_q(g, hh)

                def mx(c, m):
                    r = pl.multiple_of(c * CK, CK)
                    st = _dot(k_scr[g, pl.ds(r, CK), :], wq)
                    return jnp.maximum(m, jnp.max(st.reshape(CK // 8, 8, BQ), axis=0))
                m8 = jax.lax.fori_loop(0, NC, mx, jnp.full((8, BQ), -jnp.inf, F32))
                m = jnp.max(m8, axis=0, keepdims=True)
                acc = jnp.zeros((Dh, BQ), F32)
                lsum = jnp.zeros((8, BQ), F32)
                for c in range(NC):
                    st = _dot(k_scr[g, c * CK:(c + 1) * CK, :], wq)
                    p = jnp.exp2(st - m)
                    lsum = lsum + jnp.sum(p.reshape(CK // 8, 8, BQ), axis=0)
                    acc = acc + _dot(v_rows(g, hh, c), p.astype(BF16))
                finish(g, hh, acc, lsum)
            return carry
        jax.lax.fori_loop(0, NG, group, 0)

    r0 = pl.multiple_of(i * BQ, BQ)
    o = ot_scr[...].T.astype(BF16)
    h = x_ref[pl.ds(r0, BQ), :].astype(F32) + _dot(o, wo_ref[...])
    hn = _layernorm(h).astype(BF16)
    a = _dot(hn, w1_ref[...]) + b1_ref[...].astype(F32)
    gl = jax.nn.gelu(a, approximate=True).astype(BF16)
    y = _dot(gl, w2_ref[...]) + b2_ref[...].astype(F32)
    o_ref[...] = (h + y).astype(o_ref.dtype)


@jax.jit
def pallas_sequential_preLN__softmax_full_mha__dense_activation_gelu__prompt_kernel(
    A_x: jax.Array,
    A_wqkv: jax.Array,
    A_wo: jax.Array,
    B_x: jax.Array,
    B_w1: jax.Array,
    B_b1: jax.Array,
    B_w2: jax.Array,
    B_b2: jax.Array,
):
    del B_x
    B, S, D = A_x.shape
    assert B == 1
    F = B_w1.shape[1]
    BQ, CK, TB = 512, 256, 512
    NQ = S // BQ

    x = A_x.reshape(S, D)
    b1 = B_b1.reshape(1, F)
    b2 = B_b2.reshape(1, D)

    full = lambda shape: pl.BlockSpec(shape, lambda i: (0,) * len(shape))
    kern = functools.partial(_kernel, S=S, D=D, BQ=BQ, CK=CK, TB=TB)
    out = pl.pallas_call(
        kern,
        grid=(NQ,),
        in_specs=[full((S, D)), full((D, 3 * D)), full((D, D)), full((D, F)), full((1, F)),
                  full((F, D)), full((1, D))],
        out_specs=pl.BlockSpec((BQ, D), lambda i: (i, 0)),
        out_shape=jax.ShapeDtypeStruct((S, D), A_x.dtype),
        scratch_shapes=[
            pltpu.VMEM((D // 128, S, 128), BF16),
            pltpu.VMEM((NQ, D, BQ), BF16),
            pltpu.VMEM((D, S), BF16),
            pltpu.VMEM((D, BQ), F32),
            pltpu.SMEM((1,), jnp.int32),
        ],
        compiler_params=pltpu.CompilerParams(
            dimension_semantics=("arbitrary",),
            vmem_limit_bytes=100 * 1024 * 1024),
    )(x, A_wqkv, A_wo, B_w1, b1, B_w2, b2)
    return out.reshape(B, S, D)
```

```python
import functools
import math

import jax
import jax.numpy as jnp
import jax.experimental.pallas as pl
import jax.experimental.pallas.tpu as pltpu

F32 = jnp.float32
BF16 = jnp.bfloat16

_H = 32
_EPS = 1e-5
_LOG2E = math.log2(math.e)
_SAFE_LOG2 = 60.0
_SAFE_V = 2.0 ** 40

CFG = dict(VK=32, GATES=(4,), A=4, PF32=True, KBMODE='ssa', PIN0=0, PINS=2, PINEVERY=4)


def _layernorm(x):
    m = jnp.mean(x, axis=-1, keepdims=True)
    xc = x - m
    v = jnp.mean(xc * xc, axis=-1, keepdims=True)
    return xc * jax.lax.rsqrt(v + _EPS)


def _dot(a, b):
    return jax.lax.dot_general(a, b, (((1,), (0,)), ((), ())), preferred_element_type=F32)


def _dot_nt(a, b):
    return jax.lax.dot_general(a, b, (((1,), (1,)), ((), ())), preferred_element_type=F32)


def _kernel(x_hbm, wqkv_hbm, wo_hbm, w1_hbm, b1_ref, w2_hbm, b2_ref, o_ref,
            x_scr, wqkv_scr, wo_scr, w1_scr, w2_scr, wt_scr,
            k_scr, kf_scr, qt_scr, qf_scr, vt_scr, acc_scr, kb_scr, sv_scr, wq_scr,
            flag_ref, sems, *, S, D, BQ, CK, VK, GATES, A, PF32, KBMODE, PIN0, PINS, PINEVERY):
    H = _H
    Dh = D // H
    HG = 128 // Dh
    NG = H // HG
    NC = S // CK
    NQ = S // BQ
    CPB = BQ // CK
    NT = BQ // 128
    MK = CK - VK
    CB = 2
    i = pl.program_id(0)

    def x_copy(tb):
        return pltpu.make_async_copy(x_hbm.at[pl.ds(tb * BQ, BQ)], x_scr.at[pl.ds(tb * BQ, BQ)], sems.at[tb])
    cp_wqkv = pltpu.make_async_copy(wqkv_hbm, wqkv_scr, sems.at[NQ])
    cp_wo = pltpu.make_async_copy(wo_hbm, wo_scr, sems.at[NQ + 1])
    cp_w1 = pltpu.make_async_copy(w1_hbm, w1_scr, sems.at[NQ + 2])
    cp_w2 = pltpu.make_async_copy(w2_hbm, w2_scr, sems.at[NQ + 3])

    @pl.when(i == 0)
    def _attention():
        cp_wqkv.start()
        for tb in range(NQ):
            x_copy(tb).start()
        cp_wo.start()
        cp_w1.start()
        cp_w2.start()
        acc_scr[...] = jnp.zeros(acc_scr.shape, F32)
        cp_wqkv.wait()
        wt_scr[0:D, :] = wqkv_scr[:, 0:D].T
        wt_scr[D:2 * D, :] = wqkv_scr[:, 2 * D:3 * D].T

        qscale = (Dh ** -0.5) * _LOG2E

        def proj(tb, carry):
            qn_max, kk_max, v_max = carry
            r0 = pl.multiple_of(tb * BQ, BQ)
            pltpu.make_async_copy(x_hbm.at[pl.ds(r0, BQ)], x_scr.at[pl.ds(r0, BQ)], sems.at[tb]).wait()
            xn = _layernorm(x_scr[pl.ds(r0, BQ), :].astype(F32)).astype(BF16)
            k = _dot(xn, wqkv_scr[:, D:2 * D]).astype(BF16)
            kf = k.astype(F32)
            for g in range(NG):
                k_scr[g, pl.ds(r0, BQ), :] = k[:, g * 128:(g + 1) * 128]
                if VK:
                    for cc in range(CPB):
                        kf_scr[g, tb * CPB + cc] = kf[cc * CK + MK:(cc + 1) * CK, g * 128:(g + 1) * 128]
            qv = _dot_nt(wt_scr[...], xn)
            qt = (qv[0:D] * qscale).astype(BF16)
            qf = qt.astype(F32)
            vt = qv[D:2 * D].astype(BF16)
            qt_scr[tb] = qt.reshape(H, Dh, BQ)
            if VK:
                qf_scr[tb] = qf.reshape(H, Dh, BQ)
            for cc in range(CPB):
                vt_scr[tb * CPB + cc] = vt[:, cc * CK:(cc + 1) * CK].reshape(H, Dh, CK)
            qn_max = jnp.maximum(qn_max, jnp.sum((qf * qf).reshape(H, Dh, BQ), axis=1))
            kk_max = jnp.maximum(kk_max, jnp.max((kf * kf).reshape(8, BQ // 8, D), axis=0))
            v_max = jnp.maximum(v_max, jnp.max(jnp.abs(qv[D:2 * D]).reshape(D // 8, 8, BQ), axis=0))
            return qn_max, kk_max, v_max

        qn_max, kk_max, v_max = jax.lax.fori_loop(
            0, NQ, proj,
            (jnp.zeros((H, BQ), F32), jnp.zeros((BQ // 8, D), F32), jnp.zeros((8, BQ), F32)))
        seg = (jax.lax.broadcasted_iota(jnp.int32, (D, 128), 0) // Dh
               == jax.lax.broadcasted_iota(jnp.int32, (D, 128), 1)).astype(BF16)
        kn = _dot((kk_max * 1.02).astype(BF16), seg)
        bound2 = jnp.max(qn_max) * jnp.max(kn)
        fast = jnp.logical_and(bound2 <= _SAFE_LOG2 * _SAFE_LOG2, jnp.max(v_max) <= _SAFE_V)

        NIT = NG * (NC // CB)
        NGRP = HG * CB
        NSTEP = NGRP * NQ

        def bcast(g, c, hh, d):
            lane = hh * Dh + d
            return jnp.broadcast_to(kf_scr[g, c][:, lane:lane + 1], (VK, 128))

        def vpu_scores(kb, h, qb, state, pin=None):
            rows = []
            for g16 in range(VK // 16):
                cols = []
                for qt in range(NT):
                    gate = GATES[state['cnt'] % len(GATES)]
                    state['cnt'] += 1
                    z = pin((qb * (VK // 16) + g16) * NT + qt) if pin is not None else None
                    a = [None, None]
                    for d in range(Dh):
                        qv = jnp.broadcast_to(qf_scr[qb, h, d:d + 1, qt * 128:(qt + 1) * 128], (8, 128))
                        if d == gate and state['tok'] is not None:
                            qv = qv + state['tok']
                        if d == 0 and z is not None:
                            qv = qv + z
                        for s in range(2):
                            t = kb(d, g16 * 16 + s * 8) * qv
                            a[s] = t if a[s] is None else a[s] + t
                    u = a[0] - a[1]
                    state['tok'] = u - u
                    cols.append(a)
                for s in range(2):
                    rows.append(jnp.concatenate([cols[qt][s] for qt in range(NT)], axis=1))
            return jnp.concatenate(rows, axis=0)

        @pl.when(fast)
        def _fast():
            if VK:
                assert A == NQ
                st0 = dict(cnt=0, tok=None)
                kb0 = [bcast(0, 0, 0, d) for d in range(Dh)]
                for qb in range(NQ):
                    sv_scr[qb] = vpu_scores(lambda d, r: kb0[d][r:r + 8], 0, qb, st0)
                for grp in range(1, NGRP + 1):
                    for d in range(Dh):
                        if grp < NGRP:
                            kb_scr[0, grp - 1, d] = bcast(0, grp % CB, grp // CB, d)
                        else:
                            kb_scr[0, grp - 1, d] = bcast(0, CB, 0, d)

            def body(it, carry):
                g = it // (NC // CB)
                c0 = (it % (NC // CB)) * CB
                itn = jnp.minimum(it + 1, NIT - 1)
                gn = itn // (NC // CB)
                c0n = (itn % (NC // CB)) * CB
                seq = [(hh, cc, qb) for hh in range(HG) for cc in range(CB) for qb in range(NQ)]
                state = dict(cnt=0, tok=None)
                sv, pts, part, lsum = {}, {}, {}, {}

                it2 = jnp.minimum(it + 2, NIT - 1)
                g2 = it2 // (NC // CB)
                c02 = (it2 % (NC // CB)) * CB

                def group(grp):
                    if grp < NGRP:
                        return g, c0 + grp % CB, grp // CB
                    grp -= NGRP
                    if grp < NGRP:
                        return gn, c0n + grp % CB, grp // CB
                    grp -= NGRP
                    return g2, c02 + grp % CB, grp // CB

                def vpu(j):
                    grp, qb = j // NQ, j % NQ
                    gg, _, hh = group(grp)
                    kb = lambda d, r: kb_scr[it, grp - 1, d, r:r + 8, :]

                    def pin(idx):
                        if idx < PIN0 or (idx - PIN0) % PINS or (idx - PIN0) // PINS >= Dh:
                            return None
                        d = (idx - PIN0) // PINS
                        gb, cb, hb = group(grp + NGRP)
                        v = bcast(gb, cb, hb, d)
                        kb_scr[it + 1, grp - 1, d] = v
                        if PINEVERY == 0 or d % PINEVERY != PINEVERY - 1:
                            return None
                        w = v[0:8]
                        for r in range(8, VK, 8):
                            w = w + v[r:r + 8]
                        return w - w
                    r = vpu_scores(kb, gg * HG + hh, qb, state, pin)
                    if j >= NSTEP:
                        sv_scr[j - NSTEP] = r
                    else:
                        sv[j] = r

                def qk(j):
                    hh, cc, qb = seq[j]
                    parts = []
                    if hh > 0:
                        parts.append(jnp.zeros((hh * Dh, BQ), BF16))
                    parts.append(qt_scr[qb, g * HG + hh])
                    if hh < HG - 1:
                        parts.append(jnp.zeros(((HG - 1 - hh) * Dh, BQ), BF16))
                    wq = jnp.concatenate(parts, axis=0)
                    r0 = pl.multiple_of((c0 + cc) * CK, CK)
                    st = _dot(k_scr[g, pl.ds(r0, MK), :], wq)
                    if VK:
                        r = sv_scr[j] if j < A else sv.pop(j)
                        st = jnp.concatenate([st, r], axis=0)
                    p = jnp.exp2(st)
                    ps = jnp.sum(p.reshape(CK // 8, 8, BQ), axis=0)
                    lsum[(hh, qb)] = ps if cc == 0 else ps + lsum[(hh, qb)]
                    pts[j] = p if PF32 else p.astype(BF16)

                def pv(j):
                    hh, cc, qb = seq[j]
                    h = g * HG + hh
                    o = _dot(vt_scr[c0 + cc, h], pts.pop(j))
                    if cc == 0:
                        part[(hh, qb)] = o + acc_scr[qb, h, 0:Dh, :]
                    else:
                        part[(hh, qb)] = o + part[(hh, qb)]
                    if cc == CB - 1:
                        acc_scr[qb, h, 0:Dh, :] = part.pop((hh, qb))
                        acc_scr[qb, h, Dh:Dh + 8, :] = lsum.pop((hh, qb)) + acc_scr[qb, h, Dh:Dh + 8, :]

                for j in range(NSTEP + 1):
                    if j < NSTEP:
                        qk(j)
                        if VK:
                            vpu(j + A)
                    if j >= 1:
                        pv(j - 1)
                return carry
            jax.lax.fori_loop(0, NIT, body, 0)
            if VK:
                v = kb_scr[NIT, 0, 0, 0:8, :]
                acc_scr[0, 0, Dh:Dh + 8, 0:128] = acc_scr[0, 0, Dh:Dh + 8, 0:128] + (v - v)

        @pl.when(jnp.logical_not(fast))
        def _slow():
            def head(h, carry):
                g = h // HG
                wq_scr[...] = jnp.zeros(wq_scr.shape, BF16)
                r0 = pl.multiple_of((h % HG) * Dh, Dh)
                for qb in range(NQ):
                    wq_scr[pl.ds(r0, Dh), qb * BQ:(qb + 1) * BQ] = qt_scr[qb, h]

                def scores(c):
                    return _dot(k_scr[g, pl.ds(pl.multiple_of(c * CK, CK), CK), :], wq_scr[...])

                def mx(c, m):
                    return jnp.maximum(m, jnp.max(scores(c).reshape(CK // 8, 8, S), axis=0))
                m8 = jax.lax.fori_loop(0, NC, mx, jnp.full((8, S), -jnp.inf, F32))
                m = jnp.max(m8, axis=0, keepdims=True)

                def acc(c, carry):
                    o, l = carry
                    p = jnp.exp2(scores(c) - m)
                    return (o + _dot(vt_scr[c, h], p.astype(BF16)),
                            l + jnp.sum(p.reshape(CK // 8, 8, S), axis=0))
                o, l = jax.lax.fori_loop(0, NC, acc, (jnp.zeros((Dh, S), F32), jnp.zeros((8, S), F32)))
                for qb in range(NQ):
                    acc_scr[qb, h, 0:Dh, :] = o[:, qb * BQ:(qb + 1) * BQ]
                    acc_scr[qb, h, Dh:Dh + 8, :] = l[:, qb * BQ:(qb + 1) * BQ]
                return carry
            jax.lax.fori_loop(0, H, head, 0)

        cp_wo.wait()
        cp_w1.wait()
        cp_w2.wait()

    r0 = pl.multiple_of(i * BQ, BQ)
    a = acc_scr[i]
    l = jnp.sum(a[:, Dh:Dh + 8, :], axis=1, keepdims=True)
    ot = (a[:, 0:Dh, :] / l).reshape(D, BQ)
    o = ot.T.astype(BF16)
    h = x_scr[pl.ds(r0, BQ), :].astype(F32) + _dot(o, wo_scr[...])
    hn = _layernorm(h).astype(BF16)
    z = _dot(hn, w1_scr[...]) + b1_ref[...].astype(F32)
    gl = jax.nn.gelu(z, approximate=True).astype(BF16)
    y = _dot(gl, w2_scr[...]) + b2_ref[...].astype(F32)
    o_ref[...] = (h + y).astype(o_ref.dtype)


@jax.jit
def pallas_sequential_preLN__softmax_full_mha__dense_activation_gelu__prompt_kernel(
    A_x: jax.Array,
    A_wqkv: jax.Array,
    A_wo: jax.Array,
    B_x: jax.Array,
    B_w1: jax.Array,
    B_b1: jax.Array,
    B_w2: jax.Array,
    B_b2: jax.Array,
):
    del B_x
    B, S, D = A_x.shape
    assert B == 1
    F = B_w1.shape[1]
    BQ, CK = 512, 256
    NQ = S // BQ
    NC = S // CK
    H = _H
    Dh = D // H
    VK, A = CFG['VK'], CFG['A']
    VKp = max(VK, 8)

    x = A_x.reshape(S, D)
    b1 = B_b1.reshape(1, F)
    b2 = B_b2.reshape(1, D)

    hbm = pl.BlockSpec(memory_space=pl.ANY)
    full = lambda shape: pl.BlockSpec(shape, lambda i: (0,) * len(shape))
    kern = functools.partial(_kernel, S=S, D=D, BQ=BQ, CK=CK, **CFG)
    out = pl.pallas_call(
        kern,
        grid=(NQ,),
        in_specs=[hbm, hbm, hbm, hbm, full((1, F)), hbm, full((1, D))],
        out_specs=pl.BlockSpec((BQ, D), lambda i: (i, 0)),
        out_shape=jax.ShapeDtypeStruct((S, D), A_x.dtype),
        scratch_shapes=[
            pltpu.VMEM((S, D), BF16),
            pltpu.VMEM((D, 3 * D), BF16),
            pltpu.VMEM((D, D), BF16),
            pltpu.VMEM((D, F), BF16),
            pltpu.VMEM((F, D), BF16),
            pltpu.VMEM((2 * D, D), BF16),
            pltpu.VMEM((D // 128, S, 128), BF16),
            pltpu.VMEM((D // 128, NC, VKp, 128), F32),
            pltpu.VMEM((NQ, H, Dh, BQ), BF16),
            pltpu.VMEM((NQ, H, Dh, BQ), F32),
            pltpu.VMEM((NC, H, Dh, CK), BF16),
            pltpu.VMEM((NQ, H, Dh + 8, BQ), F32),
            pltpu.VMEM((17, 16, Dh, VKp, 128), F32),
            pltpu.VMEM((A, VKp, BQ), F32),
            pltpu.VMEM((128, S), BF16),
            pltpu.SMEM((1,), jnp.int32),
            pltpu.SemaphoreType.DMA((NQ + 4,)),
        ],
        compiler_params=pltpu.CompilerParams(
            dimension_semantics=("arbitrary",),
            vmem_limit_bytes=120 * 1024 * 1024),
    )(x, A_wqkv, A_wo, B_w1, b1, B_w2, b2)
    return out.reshape(B, S, D)
```

```python
import functools
import math

import jax
import jax.numpy as jnp
import jax.experimental.pallas as pl
import jax.experimental.pallas.tpu as pltpu

F32 = jnp.float32
BF16 = jnp.bfloat16
U32 = jnp.uint32

_H = 32
_EPS = 1e-5
_LOG2E = math.log2(math.e)
_SAFE_LOG2 = 60.0
_SAFE_V = 2.0 ** 40

CFG = dict(VK=32, GATES=(4,), PF32=True, PINS=2, PINEVERY=0, XL=(0,2,4,6,8,10,12,14), XALL=True, XWAIT=(0, 1, 2, 3), WWAIT=3, OPIPE=False, LNPOST=True, RCP=True, LN1MODE='raw', CARRY=True)
CFG.update(dict(XALL=False, XWAIT=(0, 1, 1, 3)))


def _layernorm(x):
    m = jnp.mean(x, axis=-1, keepdims=True)
    xc = x - m
    v = jnp.mean(xc * xc, axis=-1, keepdims=True)
    return xc * jax.lax.rsqrt(v + _EPS)


def _center_scale(x):
    m = jnp.mean(x, axis=-1, keepdims=True)
    xc = x - m
    v = jnp.mean(xc * xc, axis=-1, keepdims=True)
    return xc, jax.lax.rsqrt(v + _EPS)


def _dot(a, b):
    return jax.lax.dot_general(a, b, (((1,), (0,)), ((), ())), preferred_element_type=F32)


def _dot_nt(a, b):
    return jax.lax.dot_general(a, b, (((1,), (1,)), ((), ())), preferred_element_type=F32)


def _pack(a):
    return pltpu.bitcast(a.astype(BF16), U32)


def _unpack(a):
    return pltpu.bitcast(a, BF16)


def _fold_max(a):
    r, c = a.shape
    a = jnp.max(a.reshape(r // 8, 8, c), axis=0)
    m = a[:, 0:128]
    for t in range(1, c // 128):
        m = jnp.maximum(m, a[:, t * 128:(t + 1) * 128])
    return m


def _kernel(x_hbm, wqkv_hbm, wo_hbm, w1_hbm, b1_hbm, w2_hbm, b2_hbm, o_ref,
            x_scr, xn_scr, wqkv_scr, wo_scr, w1_scr, w2_scr, wt_scr,
            k_scr, kf_scr, qt_scr, qf_scr, vt_scr, acc_scr, kb_scr, sv_scr, wq_scr, on_scr, b1_scr, b2_scr, pc_scr,
            sems, *, S, D, BQ, CK, VK, GATES, PF32, PINS, PINEVERY, XL, XALL, XWAIT, WWAIT, OPIPE, LNPOST, RCP, LN1MODE, CARRY):
    H = _H
    Dh = D // H
    HG = 128 // Dh
    NG = H // HG
    NC = S // CK
    NQ = S // BQ
    CPB = BQ // CK
    NT = BQ // 128
    MK = CK - VK
    CB = 2
    NCB = NC // CB
    NIT = NG * NCB
    NGRP = HG * CB
    NSTEP = NGRP * NQ
    A = NQ
    assert VK // 8 == NQ
    i = pl.program_id(0)

    def x_copy(tb):
        return pltpu.make_async_copy(x_hbm.at[pl.ds(tb * BQ, BQ)], x_scr.at[pl.ds(tb * BQ, BQ)], sems.at[tb])

    def w_copy(j):
        return pltpu.make_async_copy(wqkv_hbm.at[:, pl.ds(j * D, D)], wqkv_scr.at[j], sems.at[NQ + j])
    cp_wo = pltpu.make_async_copy(wo_hbm, wo_scr, sems.at[NQ + 3])
    cp_w1 = pltpu.make_async_copy(w1_hbm, w1_scr, sems.at[NQ + 4])
    cp_w2 = pltpu.make_async_copy(w2_hbm, w2_scr, sems.at[NQ + 5])
    cp_b1 = pltpu.make_async_copy(b1_hbm, b1_scr, sems.at[NQ + 6])
    cp_b2 = pltpu.make_async_copy(b2_hbm, b2_scr, sems.at[NQ + 7])

    def prep_o(qb):
        a = acc_scr[qb]
        l = jnp.sum(a[:, Dh:Dh + 8, :], axis=1, keepdims=True)
        if RCP:
            inv = pl.reciprocal(l, approx=True)
            inv = inv * (2.0 - l * inv)
            ot = (a[:, 0:Dh, :] * inv).reshape(D, BQ)
        else:
            ot = (a[:, 0:Dh, :] / l).reshape(D, BQ)
        return ot.T.astype(BF16)

    def vpu_scores(kb, h, qb, state, pin=None):
        rows = []
        for g16 in range(VK // 16):
            cols = []
            for qt in range(NT):
                z = pin((qb * (VK // 16) + g16) * NT + qt) if pin is not None else None
                gate = -1
                if state is not None:
                    gate = GATES[state['cnt'] % len(GATES)]
                    state['cnt'] += 1
                a = [None, None]
                for d in range(Dh):
                    qv = jnp.broadcast_to(qf_scr[qb, h, d:d + 1, qt * 128:(qt + 1) * 128], (8, 128))
                    if d == gate and state['tok'] is not None:
                        qv = qv + state['tok']
                    if d == 0 and z is not None:
                        qv = qv + z
                    for s in range(2):
                        t = kb(d, g16 * 16 + s * 8) * qv
                        a[s] = t if a[s] is None else a[s] + t
                if state is not None:
                    u = a[0] - a[1]
                    state['tok'] = u - u
                cols.append(a)
            for s in range(2):
                rows.append(jnp.concatenate([cols[qt][s] for qt in range(NT)], axis=1))
        return jnp.concatenate(rows, axis=0)

    @pl.when(i == 0)
    def _attention():
        w_copy(1).start()
        for tb in range(NQ):
            x_copy(tb).start()
        w_copy(0).start()
        w_copy(2).start()
        cp_wo.start()
        cp_w1.start()
        cp_w2.start()
        cp_b1.start()
        cp_b2.start()
        acc_scr[...] = jnp.zeros(acc_scr.shape, F32)
        pc_scr[...] = jnp.zeros(pc_scr.shape, F32)

        w_copy(1).wait()
        kk_max = None
        for tb in range(NQ):
            for t2 in range(NQ):
                if XWAIT[t2] == tb:
                    x_copy(t2).wait()
            if tb == WWAIT:
                w_copy(0).wait()
                w_copy(2).wait()
                wt_scr[0:D, :] = wqkv_scr[0].T
                wt_scr[D:2 * D, :] = wqkv_scr[2].T
            rows = slice(tb * BQ, (tb + 1) * BQ)
            if LN1MODE == 'raw':
                xb = x_scr[rows, :]
                xf = xb.astype(F32)
                m = jnp.mean(xf, axis=-1, keepdims=True)
                xc = xf - m
                r = jax.lax.rsqrt(jnp.mean(xc * xc, axis=-1, keepdims=True) + _EPS)
                xn_scr[tb] = (xc * r).astype(BF16)
                if tb == 0:
                    wk_cs = _dot(jnp.ones((8, D), BF16), wqkv_scr[1])[0:1]
                kf = ((_dot(xb, wqkv_scr[1]) - m * wk_cs) * r).astype(BF16).astype(F32)
            elif LN1MODE == 'post':
                xc, r = _center_scale(x_scr[rows, :].astype(F32))
                xn_scr[tb] = (xc * r).astype(BF16)
                kf = (_dot(xc.astype(BF16), wqkv_scr[1]) * r).astype(BF16).astype(F32)
            else:
                xn = _layernorm(x_scr[rows, :].astype(F32)).astype(BF16)
                xn_scr[tb] = xn
                kf = _dot(xn, wqkv_scr[1]).astype(BF16).astype(F32)
            for g in range(NG):
                k_scr[g, tb * BQ // 2:(tb + 1) * BQ // 2, :] = _pack(kf[:, g * 128:(g + 1) * 128])
                for cc in range(CPB):
                    kf_scr[g, tb * CPB + cc] = kf[cc * CK + MK:(cc + 1) * CK, g * 128:(g + 1) * 128]
            kk = jnp.max((kf * kf).reshape(8, BQ // 8, D), axis=0)
            kk_max = kk if kk_max is None else jnp.maximum(kk_max, kk)
        for d in range(Dh):
            kb_scr[NIT, 0, d] = jnp.broadcast_to(kf_scr[0, 0][:, d:d + 1], (VK, 128))
        seg = (jax.lax.broadcasted_iota(jnp.int32, (D, 128), 0) // Dh
               == jax.lax.broadcasted_iota(jnp.int32, (D, 128), 1)).astype(BF16)
        kn_max = jnp.max(_dot((kk_max * 1.02).astype(BF16), seg))

        qscale = (Dh ** -0.5) * _LOG2E

        def proj(tb, carry):
            qn_max, v_max = carry
            qv = _dot_nt(wt_scr[...], xn_scr[tb])
            qf = (qv[0:D] * qscale).astype(BF16).astype(F32)
            qt_scr[tb] = _pack(qf).reshape(H, Dh // 2, BQ)
            qf_scr[tb] = qf.reshape(H, Dh, BQ)
            for cc in range(CPB):
                vt_scr[tb * CPB + cc] = _pack(qv[D:2 * D, cc * CK:(cc + 1) * CK]).reshape(H, Dh // 2, CK)
            qn_max = jnp.maximum(qn_max, _fold_max(jnp.sum((qf * qf).reshape(H, Dh, BQ), axis=1)))
            v_max = jnp.maximum(v_max, _fold_max(jnp.abs(qv[D:2 * D])))
            sv_scr[tb] = vpu_scores(lambda d, r: kb_scr[NIT, 0, d, r:r + 8, :], 0, tb, None)
            r8 = pl.multiple_of(tb * 8, 8)
            for grp in range(1, NGRP + 1):
                c, hh = (grp % CB, grp // CB) if grp < NGRP else (CB, 0)
                kv = kf_scr[0, c, pl.ds(r8, 8), :]
                for d in range(Dh):
                    lane = hh * Dh + d
                    kb_scr[0, grp - 1, d, pl.ds(r8, 8), :] = jnp.broadcast_to(kv[:, lane:lane + 1], (8, 128))
            return qn_max, v_max

        qn_max, v_max = jax.lax.fori_loop(0, NQ, proj, (jnp.zeros((8, 128), F32), jnp.zeros((8, 128), F32)))
        bound2 = jnp.max(qn_max) * kn_max
        fast = jnp.logical_and(bound2 <= _SAFE_LOG2 * _SAFE_LOG2, jnp.max(v_max) <= _SAFE_V)

        def pv_carry(t):
            h = (t // NCB) * HG + HG - 1
            c = (t % NCB) * CB + CB - 1
            o = _dot(_unpack(vt_scr[c, h]), pc_scr[...])
            acc_scr[NQ - 1, h, 0:Dh, :] = o + acc_scr[NQ - 1, h, 0:Dh, :]

        @pl.when(fast)
        def _fast():
            def body(it, carry):
                its = [it, jnp.minimum(it + 1, NIT - 1), jnp.minimum(it + 2, NIT - 1)]
                gs = [t // NCB for t in its]
                cs = [(t % NCB) * CB for t in its]
                g, c0 = gs[0], cs[0]
                seq = [(hh, cc, qb) for hh in range(HG) for cc in range(CB) for qb in range(NQ)]
                state = dict(cnt=0, tok=None)
                sv, pts, part, lsum = {}, {}, {}, {}

                def group(grp):
                    b, r = grp // NGRP, grp % NGRP
                    return gs[b], cs[b] + r % CB, r // CB

                def vpu(j):
                    grp, qb = j // NQ, j % NQ
                    gg, _, hh = group(grp)

                    def pin(idx):
                        if idx % PINS or idx // PINS >= Dh:
                            return None
                        d = idx // PINS
                        gb, cb, hb = group(grp + NGRP)
                        lane = hb * Dh + d
                        if d in XL:
                            kv = kf_scr[gb, cb]
                            xt = state.get('xtok')
                            if xt is not None:
                                if XALL:
                                    kv = kv + jnp.concatenate([xt] * (VK // 8), axis=0)
                                else:
                                    kv = jnp.concatenate([kv[0:8] + xt, kv[8:]], axis=0)
                            state['kv'] = kv
                        kv = state['kv'] if (XALL or d in XL) else kf_scr[gb, cb]
                        v = jnp.broadcast_to(kv[:, lane:lane + 1], (VK, 128))
                        kb_scr[it + 1, grp - 1, d] = v
                        if XALL and ((d + 1) % Dh) in XL:
                            w = v[VK - 8:VK]
                            state['xtok'] = w - w
                        if not XALL and d in XL:
                            w = v[0:8]
                            state['xtok'] = w - w
                        if PINEVERY == 0 or d % PINEVERY != PINEVERY - 1:
                            return None
                        w = v[0:8]
                        for r in range(8, VK, 8):
                            w = w + v[r:r + 8]
                        return w - w
                    r = vpu_scores(lambda d, r: kb_scr[it, grp - 1, d, r:r + 8, :], gg * HG + hh, qb, state, pin)
                    if j >= NSTEP:
                        sv_scr[j - NSTEP] = r
                    else:
                        sv[j] = r

                def qk(j):
                    hh, cc, qb = seq[j]
                    parts = []
                    if hh > 0:
                        parts.append(jnp.zeros((hh * Dh, BQ), BF16))
                    parts.append(_unpack(qt_scr[qb, g * HG + hh]))
                    if hh < HG - 1:
                        parts.append(jnp.zeros(((HG - 1 - hh) * Dh, BQ), BF16))
                    wq = jnp.concatenate(parts, axis=0)
                    r0 = pl.multiple_of((c0 + cc) * (CK // 2), CK // 2)
                    st = _dot(_unpack(k_scr[g, pl.ds(r0, MK // 2), :]), wq)
                    r = sv_scr[j] if j < A else sv.pop(j)
                    p = jnp.exp2(jnp.concatenate([st, r], axis=0))
                    ps = jnp.sum(p.reshape(CK // 8, 8, BQ), axis=0)
                    lsum[(hh, qb)] = ps if cc == 0 else ps + lsum[(hh, qb)]
                    pts[j] = p if PF32 else p.astype(BF16)

                def pv(j):
                    hh, cc, qb = seq[j]
                    h = g * HG + hh
                    last = CARRY and (hh, qb) == (HG - 1, NQ - 1)
                    o = _dot(_unpack(vt_scr[c0 + cc, h]), pts.pop(j))
                    if cc == 0:
                        part[(hh, qb)] = o + acc_scr[qb, h, 0:Dh, :]
                    else:
                        part[(hh, qb)] = o + part[(hh, qb)]
                    if cc == CB - 1 - (1 if last else 0):
                        acc_scr[qb, h, 0:Dh, :] = part.pop((hh, qb))
                    if cc == CB - 1:
                        acc_scr[qb, h, Dh:Dh + 8, :] = lsum.pop((hh, qb)) + acc_scr[qb, h, Dh:Dh + 8, :]

                for j in range(NSTEP + 1):
                    if j < NSTEP:
                        qk(j)
                        vpu(j + A)
                    if CARRY and j == 0:
                        pv_carry(jnp.maximum(it - 1, 0))
                    elif CARRY and j == NSTEP:
                        pc_scr[...] = pts.pop(j - 1)
                        h = g * HG + HG - 1
                        acc_scr[NQ - 1, h, Dh:Dh + 8, :] = (lsum.pop((HG - 1, NQ - 1))
                                                            + acc_scr[NQ - 1, h, Dh:Dh + 8, :])
                    elif j >= 1:
                        pv(j - 1)
                return carry
            jax.lax.fori_loop(0, NIT, body, 0)
            if CARRY:
                pv_carry(NIT - 1)
            v = kb_scr[NIT, 0, 0, 0:8, :]
            acc_scr[0, 0, Dh:Dh + 8, 0:128] = acc_scr[0, 0, Dh:Dh + 8, 0:128] + (v - v)

        @pl.when(jnp.logical_not(fast))
        def _slow():
            def head(h, carry):
                g = h // HG
                wq_scr[...] = jnp.zeros(wq_scr.shape, U32)
                r0 = pl.multiple_of((h % HG) * (Dh // 2), Dh // 2)
                for qb in range(NQ):
                    wq_scr[pl.ds(r0, Dh // 2), qb * BQ:(qb + 1) * BQ] = qt_scr[qb, h]

                def scores(c):
                    kc = k_scr[g, pl.ds(pl.multiple_of(c * (CK // 2), CK // 2), CK // 2), :]
                    return _dot(_unpack(kc), _unpack(wq_scr[...]))

                def mx(c, m):
                    return jnp.maximum(m, jnp.max(scores(c).reshape(CK // 8, 8, S), axis=0))
                m8 = jax.lax.fori_loop(0, NC, mx, jnp.full((8, S), -jnp.inf, F32))
                m = jnp.max(m8, axis=0, keepdims=True)

                def acc(c, carry):
                    o, l = carry
                    p = jnp.exp2(scores(c) - m)
                    return (o + _dot(_unpack(vt_scr[c, h]), p.astype(BF16)),
                            l + jnp.sum(p.reshape(CK // 8, 8, S), axis=0))
                o, l = jax.lax.fori_loop(0, NC, acc, (jnp.zeros((Dh, S), F32), jnp.zeros((8, S), F32)))
                for qb in range(NQ):
                    acc_scr[qb, h, 0:Dh, :] = o[:, qb * BQ:(qb + 1) * BQ]
                    acc_scr[qb, h, Dh:Dh + 8, :] = l[:, qb * BQ:(qb + 1) * BQ]
                return carry
            jax.lax.fori_loop(0, H, head, 0)

        cp_wo.wait()
        cp_w1.wait()
        cp_w2.wait()
        cp_b1.wait()
        cp_b2.wait()
        if OPIPE:
            on_scr[...] = prep_o(0)

    r0 = pl.multiple_of(i * BQ, BQ)
    o = on_scr[...] if OPIPE else prep_o(i)
    h = x_scr[pl.ds(r0, BQ), :].astype(F32) + _dot(o, wo_scr[...])
    if OPIPE:
        on_scr[...] = prep_o(jnp.minimum(i + 1, NQ - 1))
    if LNPOST:
        hc, r = _center_scale(h)
        z = _dot(hc.astype(BF16), w1_scr[...]) * r + b1_scr[...].astype(F32)[None, :]
    else:
        z = _dot(_layernorm(h).astype(BF16), w1_scr[...]) + b1_scr[...].astype(F32)[None, :]
    gl = jax.nn.gelu(z, approximate=True).astype(BF16)
    y = _dot(gl, w2_scr[...]) + b2_scr[...].astype(F32)[None, :]
    o_ref[...] = (h + y).astype(o_ref.dtype)


@jax.jit
def pallas_sequential_preLN__softmax_full_mha__dense_activation_gelu__prompt_kernel(
    A_x: jax.Array,
    A_wqkv: jax.Array,
    A_wo: jax.Array,
    B_x: jax.Array,
    B_w1: jax.Array,
    B_b1: jax.Array,
    B_w2: jax.Array,
    B_b2: jax.Array,
):
    del B_x
    B, S, D = A_x.shape
    assert B == 1
    F = B_w1.shape[1]
    BQ, CK = 512, 256
    NQ = S // BQ
    NC = S // CK
    H = _H
    Dh = D // H
    VK = CFG['VK']
    NIT = (D // 128) * (NC // 2)
    NGRP = (128 // Dh) * 2

    x = A_x.reshape(S, D)

    hbm = pl.BlockSpec(memory_space=pl.ANY)
    full = lambda shape: pl.BlockSpec(shape, lambda i: (0,) * len(shape))
    kern = functools.partial(_kernel, S=S, D=D, BQ=BQ, CK=CK, **CFG)
    out = pl.pallas_call(
        kern,
        grid=(NQ,),
        in_specs=[hbm] * 7,
        out_specs=pl.BlockSpec((BQ, D), lambda i: (i, 0)),
        out_shape=jax.ShapeDtypeStruct((S, D), A_x.dtype),
        scratch_shapes=[
            pltpu.VMEM((S, D), BF16),
            pltpu.VMEM((NQ, BQ, D), BF16),
            pltpu.VMEM((3, D, D), BF16),
            pltpu.VMEM((D, D), BF16),
            pltpu.VMEM((D, F), BF16),
            pltpu.VMEM((F, D), BF16),
            pltpu.VMEM((2 * D, D), BF16),
            pltpu.VMEM((D // 128, S // 2, 128), U32),
            pltpu.VMEM((D // 128, NC, VK, 128), F32),
            pltpu.VMEM((NQ, H, Dh // 2, BQ), U32),
            pltpu.VMEM((NQ, H, Dh, BQ), F32),
            pltpu.VMEM((NC, H, Dh // 2, CK), U32),
            pltpu.VMEM((NQ, H, Dh + 8, BQ), F32),
            pltpu.VMEM((NIT + 1, NGRP, Dh, VK, 128), F32),
            pltpu.VMEM((NQ, VK, BQ), F32),
            pltpu.VMEM((64, S), U32),
            pltpu.VMEM((BQ, D), BF16),
            pltpu.VMEM((F,), BF16),
            pltpu.VMEM((D,), BF16),
            pltpu.VMEM((CK, BQ), F32),
            pltpu.SemaphoreType.DMA((NQ + 8,)),
        ],
        compiler_params=pltpu.CompilerParams(
            dimension_semantics=("arbitrary",),
            vmem_limit_bytes=120 * 1024 * 1024),
    )(x, A_wqkv, A_wo, B_w1, B_b1, B_w2, B_b2)
    return out.reshape(B, S, D)
```

```python
import functools
import math

import jax
import jax.numpy as jnp
import jax.experimental.pallas as pl
import jax.experimental.pallas.tpu as pltpu

F32 = jnp.float32
BF16 = jnp.bfloat16
U32 = jnp.uint32

_H = 32
_EPS = 1e-5
_LOG2E = math.log2(math.e)
_SAFE_LOG2 = 60.0
_SAFE_V = 2.0 ** 40

CFG = dict(VK=32, GATES=(2,), PF32=True, XL=(0,3,5,7,9,11,13), QVU=4, CB=2, RB=128, EB=512, JOB8=False, PORD='g16', REV=0, TOK='sel', SUMV='last', XB=(0, 512, 1536, 2048), WROW=1536, OPIPE=False, LNPOST=True, RCP=True, LN1MODE='raw', CARRY=True)
CFG.update({})


def _layernorm(x):
    m = jnp.mean(x, axis=-1, keepdims=True)
    xc = x - m
    v = jnp.mean(xc * xc, axis=-1, keepdims=True)
    return xc * jax.lax.rsqrt(v + _EPS)


def _center_scale(x):
    m = jnp.mean(x, axis=-1, keepdims=True)
    xc = x - m
    v = jnp.mean(xc * xc, axis=-1, keepdims=True)
    return xc, jax.lax.rsqrt(v + _EPS)


def _dot(a, b):
    return jax.lax.dot_general(a, b, (((1,), (0,)), ((), ())), preferred_element_type=F32)


def _dot_nt(a, b):
    return jax.lax.dot_general(a, b, (((1,), (1,)), ((), ())), preferred_element_type=F32)


def _pack(a):
    return pltpu.bitcast(a.astype(BF16), U32)


def _unpack(a):
    return pltpu.bitcast(a, BF16)


def _fold_max(a):
    r, c = a.shape
    a = jnp.max(a.reshape(r // 8, 8, c), axis=0)
    m = a[:, 0:128]
    for t in range(1, c // 128):
        m = jnp.maximum(m, a[:, t * 128:(t + 1) * 128])
    return m


def _kernel(x_hbm, wqkv_hbm, wo_hbm, w1_hbm, b1_hbm, w2_hbm, b2_hbm, o_ref,
            x_scr, xn_scr, wqkv_scr, wo_scr, w1_scr, w2_scr, wt_scr,
            k_scr, kf_scr, qt_scr, qf_scr, vt_scr, acc_scr, kb_scr, sv_scr, wq_scr, on_scr, b1_scr, b2_scr, pc_scr, qg_scr,
            sems, *, S, D, BQ, CK, VK, GATES, PF32, XL, QVU, CB, RB, EB, JOB8, PORD, REV, TOK, SUMV, XB, WROW, OPIPE, LNPOST, RCP, LN1MODE, CARRY):
    H = _H
    Dh = D // H
    HG = 128 // Dh
    NG = H // HG
    NC = S // CK
    NQ = S // BQ
    CPB = BQ // CK
    NT = BQ // 128
    MK = CK - VK
    NCB = NC // CB
    NIT = NG * NCB
    NGRP = HG * CB
    NSTEP = NGRP * NQ
    A = NQ
    assert VK // 8 == NQ
    i = pl.program_id(0)

    def x_copy(j):
        rows = pl.ds(XB[j], XB[j + 1] - XB[j])
        return pltpu.make_async_copy(x_hbm.at[rows], x_scr.at[rows], sems.at[8 + j])

    def w_copy(j):
        return pltpu.make_async_copy(wqkv_hbm.at[:, pl.ds(j * D, D)], wqkv_scr.at[j], sems.at[j])
    cp_wo = pltpu.make_async_copy(wo_hbm, wo_scr, sems.at[3])
    cp_w1 = pltpu.make_async_copy(w1_hbm, w1_scr, sems.at[4])
    cp_w2 = pltpu.make_async_copy(w2_hbm, w2_scr, sems.at[5])
    cp_b1 = pltpu.make_async_copy(b1_hbm, b1_scr, sems.at[6])
    cp_b2 = pltpu.make_async_copy(b2_hbm, b2_scr, sems.at[7])

    def prep_o(qb):
        a = acc_scr[qb]
        l = jnp.sum(a[:, Dh:Dh + 8, :], axis=1, keepdims=True)
        if RCP:
            inv = pl.reciprocal(l, approx=True)
            inv = inv * (2.0 - l * inv)
            ot = (a[:, 0:Dh, :] * inv).reshape(D, BQ)
        else:
            ot = (a[:, 0:Dh, :] / l).reshape(D, BQ)
        return ot.T.astype(BF16)

    def vpu_scores(kb, h, qb, state, pin=None):
        order = [(g16, qt) for g16 in range(VK // 16) for qt in range(NT)]
        if PORD == 'qt':
            order = [(g16, qt) for qt in range(NT) for g16 in range(VK // 16)]
        res = {}
        for n, (g16, qt) in enumerate(order):
            if pin is not None:
                pin(qb * len(order) + n)
            gate = -1
            if state is not None:
                gate = GATES[state['cnt'] % len(GATES)]
                state['cnt'] += 1
            a = [None, None]
            for d in range(Dh):
                qv = jnp.broadcast_to(qf_scr[qb, h, d:d + 1, qt * 128:(qt + 1) * 128], (8, 128))
                if d == gate and state['tok'] is not None:
                    if TOK == 'sel':
                        q2 = jnp.broadcast_to(qg_scr[qb, h, d:d + 1, qt * 128:(qt + 1) * 128], (8, 128))
                        qv = jnp.where(state['tok'], qv, q2)
                    else:
                        qv = qv + state['tok']
                for s in range(2):
                    t = kb(d, g16 * 16 + s * 8) * qv
                    a[s] = t if a[s] is None else a[s] + t
            if state is not None:
                if TOK == 'sel':
                    state['tok'] = a[0] > a[1]
                elif TOK == 'a0':
                    state['tok'] = a[0] - a[0]
                elif TOK == 'alt':
                    w = a[state['cnt'] % 2]
                    state['tok'] = w - w
                else:
                    u = a[0] - a[1]
                    state['tok'] = u - u
            res[(g16, qt)] = a
        rows = [jnp.concatenate([res[(g16, qt)][s] for qt in range(NT)], axis=1)
                for g16 in range(VK // 16) for s in range(2)]
        return jnp.concatenate(rows, axis=0)

    @pl.when(i == 0)
    def _attention():
        w_copy(1).start()
        for j in range(len(XB) - 1):
            x_copy(j).start()
        w_copy(0).start()
        w_copy(2).start()
        cp_wo.start()
        cp_w1.start()
        cp_w2.start()
        cp_b1.start()
        cp_b2.start()
        acc_scr[...] = jnp.zeros(acc_scr.shape, F32)
        pc_scr[...] = jnp.zeros(pc_scr.shape, F32)

        w_copy(1).wait()
        kk_max = None
        for tb in range(NQ):
            if tb == 0:
                wk_cs = _dot(jnp.ones((8, D), BF16), wqkv_scr[1])[0:1]
            for sb in range(BQ // RB):
                t0 = tb * BQ + sb * RB
                if t0 in XB:
                    x_copy(XB.index(t0)).wait()
                if t0 == WROW:
                    w_copy(0).wait()
                    w_copy(2).wait()
                    wt_scr[0:D, :] = wqkv_scr[0].T
                    wt_scr[D:2 * D, :] = wqkv_scr[2].T
                xb = x_scr[t0:t0 + RB, :]
                xf = xb.astype(F32)
                m = jnp.mean(xf, axis=-1, keepdims=True)
                xc = xf - m
                r = jax.lax.rsqrt(jnp.mean(xc * xc, axis=-1, keepdims=True) + _EPS)
                xn_scr[tb, sb * RB:(sb + 1) * RB, :] = (xc * r).astype(BF16)
                kf = (_dot(xb, wqkv_scr[1]) - m * wk_cs) * r
                for g in range(NG):
                    k_scr[g, t0 // 2:(t0 + RB) // 2, :] = _pack(kf[:, g * 128:(g + 1) * 128])
                    for c in range(NC):
                        lo, hi = c * CK + MK - t0, (c + 1) * CK - t0
                        if lo >= 0 and hi <= RB:
                            kf_scr[g, c] = kf[lo:hi, g * 128:(g + 1) * 128].astype(BF16).astype(F32)
                kk = jnp.max((kf * kf).reshape(RB // 64, 64, D), axis=0)
                kk_max = kk if kk_max is None else jnp.maximum(kk_max, kk)
        for d in range(Dh):
            kb_scr[NIT, 0, d] = jnp.broadcast_to(kf_scr[0, 0][:, d:d + 1], (VK, 128))
        seg = (jax.lax.broadcasted_iota(jnp.int32, (D, 128), 0) // Dh
               == jax.lax.broadcasted_iota(jnp.int32, (D, 128), 1)).astype(BF16)
        kn_max = jnp.max(_dot((kk_max * 1.03).astype(BF16), seg))

        qscale = (Dh ** -0.5) * _LOG2E

        def proj(tb, carry):
            qn_max, v_max = carry
            qv = _dot_nt(wt_scr[...], xn_scr[tb])
            qf = (qv[0:D] * qscale).astype(BF16).astype(F32)
            qt_scr[tb] = _pack(qf).reshape(H, Dh // 2, BQ)
            qf_scr[tb] = qf.reshape(H, Dh, BQ)
            if TOK == 'sel':
                qg_scr[tb] = qf.reshape(H, Dh, BQ)[:, 0:8, :]
            for cc in range(CPB):
                vt_scr[tb * CPB + cc] = _pack(qv[D:2 * D, cc * CK:(cc + 1) * CK]).reshape(H, Dh // 2, CK)
            qn_max = jnp.maximum(qn_max, _fold_max(jnp.sum((qf * qf).reshape(H, Dh, BQ), axis=1)))
            v_max = jnp.maximum(v_max, _fold_max(jnp.abs(qv[D:2 * D])))
            sv_scr[tb] = vpu_scores(lambda d, r: kb_scr[NIT, 0, d, r:r + 8, :], 0, tb, None)
            r8 = pl.multiple_of(tb * 8, 8)
            for grp in range(1, NGRP + 1):
                c, hh = (grp % CB, grp // CB) if grp < NGRP else (CB, 0)
                kv = kf_scr[0, c, pl.ds(r8, 8), :]
                for d in range(Dh):
                    lane = hh * Dh + d
                    kb_scr[0, grp - 1, d, pl.ds(r8, 8), :] = jnp.broadcast_to(kv[:, lane:lane + 1], (8, 128))
            return qn_max, v_max

        qn_max, v_max = jax.lax.fori_loop(0, NQ, proj, (jnp.zeros((8, 128), F32), jnp.zeros((8, 128), F32)), unroll=QVU)
        bound2 = jnp.max(qn_max) * kn_max
        fast = jnp.logical_and(bound2 <= _SAFE_LOG2 * _SAFE_LOG2, jnp.max(v_max) <= _SAFE_V)

        def pv_carry(t):
            h = (t // NCB) * HG + HG - 1
            c = (t % NCB) * CB + CB - 1
            o = _dot(_unpack(vt_scr[c, h]), pc_scr[...])
            acc_scr[NQ - 1, h, 0:Dh, :] = o + acc_scr[NQ - 1, h, 0:Dh, :]

        @pl.when(fast)
        def _fast():
            def body(it, carry):
                its = [it, jnp.minimum(it + 1, NIT - 1), jnp.minimum(it + 2, NIT - 1)]
                gs = [t // NCB for t in its]
                cs = [(t % NCB) * CB for t in its]
                g, c0 = gs[0], cs[0]
                seq = [(hh, cc, qb) for hh in range(HG) for cc in range(CB) for qb in range(NQ)]
                state = dict(cnt=0, tok=None)
                sv, pts, part, lsum = {}, {}, {}, {}

                def group(grp):
                    b, r = grp // NGRP, grp % NGRP
                    return gs[b], cs[b] + r % CB, r // CB

                def vpu(j):
                    grp, qb = j // NQ, j % NQ
                    gg, _, hh = group(grp)

                    def bc(grps, d, link):
                        for n, gr in enumerate(grps):
                            gb, cb, hb = group(gr + NGRP)
                            lane = hb * Dh + d
                            kv = kf_scr[gb, cb]
                            xt = state.get('xtok')
                            if link and n == 0 and xt is not None:
                                kv = jnp.concatenate([kv[0:8] + xt, kv[8:]], axis=0)
                            v = jnp.broadcast_to(kv[:, lane:lane + 1], (VK, 128))
                            kb_scr[it + 1, gr - 1, d] = v
                            if link and n == 0:
                                w = v[0:8]
                                state['xtok'] = w - w

                    def pin(idx):
                        if JOB8:
                            if idx % 4:
                                return
                            hb = (grp - 1) // 2
                            d = ((grp - 1) % 2) * (Dh // 2) + idx // 4
                            bc((2 * hb + 1, 2 * hb if hb else NGRP), d, True)
                        else:
                            if idx % 2:
                                return
                            bc((grp,), idx // 2, (idx // 2) in XL)
                    r = vpu_scores(lambda d, r: kb_scr[it, grp - 1, d, r:r + 8, :], gg * HG + hh, qb, state, pin)
                    if j >= NSTEP:
                        sv_scr[j - NSTEP] = r
                    else:
                        sv[j] = r

                def qk(j):
                    hh, cc, qb = seq[j]
                    parts = []
                    if hh > 0:
                        parts.append(jnp.zeros((hh * Dh, BQ), BF16))
                    parts.append(_unpack(qt_scr[qb, g * HG + hh]))
                    if hh < HG - 1:
                        parts.append(jnp.zeros(((HG - 1 - hh) * Dh, BQ), BF16))
                    wq = jnp.concatenate(parts, axis=0)
                    r0 = pl.multiple_of((c0 + cc) * (CK // 2), CK // 2)
                    r = sv_scr[j] if j < A else sv.pop(j)
                    if REV:
                        n16 = MK // 16
                        if REV == 1:
                            perm = [7 - p if p < 8 else n16 + 7 - p for p in range(n16)]
                        else:
                            perm = [p if p < 8 else n16 + 7 - p for p in range(n16)]
                        kc = jnp.concatenate([k_scr[g, pl.ds(r0 + 8 * p, 8), :] for p in perm], axis=0)
                        st = _dot(_unpack(kc), wq)
                    else:
                        st = _dot(_unpack(k_scr[g, pl.ds(r0, MK // 2), :]), wq)
                    if SUMV == 'last':
                        p = jnp.exp2(jnp.concatenate([st, r], axis=0))
                        ps = jnp.sum(p.reshape(CK // 8, 8, BQ), axis=0)
                    elif SUMV == 'first':
                        p = jnp.exp2(jnp.concatenate([r, st], axis=0))
                        ps = jnp.sum(p.reshape(CK // 8, 8, BQ), axis=0)
                        p = jnp.concatenate([p[VK:], p[:VK]], axis=0)
                    else:
                        p = jnp.exp2(jnp.concatenate([st[:128], r, st[128:]], axis=0))
                        ps = jnp.sum(p.reshape(CK // 8, 8, BQ), axis=0)
                        p = jnp.concatenate([p[:128], p[128 + VK:], p[128:128 + VK]], axis=0)
                    if REV:
                        inv = [perm.index(q) for q in range(n16)]
                        p = jnp.concatenate([p[16 * q:16 * q + 16] for q in inv] + [p[MK:]], axis=0)
                    lsum[(hh, qb)] = ps if cc == 0 else ps + lsum[(hh, qb)]
                    pts[j] = p if PF32 else p.astype(BF16)

                def pv(j):
                    hh, cc, qb = seq[j]
                    h = g * HG + hh
                    last = CARRY and (hh, qb) == (HG - 1, NQ - 1)
                    o = _dot(_unpack(vt_scr[c0 + cc, h]), pts.pop(j))
                    if cc == 0:
                        part[(hh, qb)] = o + acc_scr[qb, h, 0:Dh, :]
                    else:
                        part[(hh, qb)] = o + part[(hh, qb)]
                    if cc == CB - 1 - (1 if last else 0):
                        acc_scr[qb, h, 0:Dh, :] = part.pop((hh, qb))
                    if cc == CB - 1:
                        acc_scr[qb, h, Dh:Dh + 8, :] = lsum.pop((hh, qb)) + acc_scr[qb, h, Dh:Dh + 8, :]

                for j in range(NSTEP + 1):
                    if j < NSTEP:
                        qk(j)
                        vpu(j + A)
                    if CARRY and j == 0:
                        pv_carry(jnp.maximum(it - 1, 0))
                    elif CARRY and j == NSTEP:
                        pc_scr[...] = pts.pop(j - 1)
                        h = g * HG + HG - 1
                        acc_scr[NQ - 1, h, Dh:Dh + 8, :] = (lsum.pop((HG - 1, NQ - 1))
                                                            + acc_scr[NQ - 1, h, Dh:Dh + 8, :])
                    elif j >= 1:
                        pv(j - 1)
                return carry
            jax.lax.fori_loop(0, NIT, body, 0)
            if CARRY:
                pv_carry(NIT - 1)
            v = kb_scr[NIT, 0, 0, 0:8, :]
            acc_scr[0, 0, Dh:Dh + 8, 0:128] = acc_scr[0, 0, Dh:Dh + 8, 0:128] + (v - v)

        @pl.when(jnp.logical_not(fast))
        def _slow():
            def head(h, carry):
                g = h // HG
                wq_scr[...] = jnp.zeros(wq_scr.shape, U32)
                r0 = pl.multiple_of((h % HG) * (Dh // 2), Dh // 2)
                for qb in range(NQ):
                    wq_scr[pl.ds(r0, Dh // 2), qb * BQ:(qb + 1) * BQ] = qt_scr[qb, h]

                def scores(c):
                    kc = k_scr[g, pl.ds(pl.multiple_of(c * (CK // 2), CK // 2), CK // 2), :]
                    return _dot(_unpack(kc), _unpack(wq_scr[...]))

                def mx(c, m):
                    return jnp.maximum(m, jnp.max(scores(c).reshape(CK // 8, 8, S), axis=0))
                m8 = jax.lax.fori_loop(0, NC, mx, jnp.full((8, S), -jnp.inf, F32))
                m = jnp.max(m8, axis=0, keepdims=True)

                def acc(c, carry):
                    o, l = carry
                    p = jnp.exp2(scores(c) - m)
                    return (o + _dot(_unpack(vt_scr[c, h]), p.astype(BF16)),
                            l + jnp.sum(p.reshape(CK // 8, 8, S), axis=0))
                o, l = jax.lax.fori_loop(0, NC, acc, (jnp.zeros((Dh, S), F32), jnp.zeros((8, S), F32)))
                for qb in range(NQ):
                    acc_scr[qb, h, 0:Dh, :] = o[:, qb * BQ:(qb + 1) * BQ]
                    acc_scr[qb, h, Dh:Dh + 8, :] = l[:, qb * BQ:(qb + 1) * BQ]
                return carry
            jax.lax.fori_loop(0, H, head, 0)

        cp_wo.wait()
        cp_w1.wait()
        cp_w2.wait()
        cp_b1.wait()
        cp_b2.wait()
        if OPIPE:
            on_scr[...] = prep_o(0)

    o = prep_o(i)
    b1 = b1_scr[...].astype(F32)[None, :]
    b2 = b2_scr[...].astype(F32)[None, :]
    hs, gs_ = [], []
    nsb = BQ // EB
    for sb in range(nsb):
        r0 = pl.multiple_of(i * BQ + sb * EB, EB)
        hs.append(x_scr[pl.ds(r0, EB), :].astype(F32) + _dot(o[sb * EB:(sb + 1) * EB], wo_scr[...]))
    def ffn1(sb):
        hc, r = _center_scale(hs[sb])
        z = _dot(hc.astype(BF16), w1_scr[...]) * r + b1
        gs_.append(jax.nn.gelu(z, approximate=True).astype(BF16))
    def ffn2(sb):
        y = _dot(gs_[sb], w2_scr[...]) + b2
        o_ref[sb * EB:(sb + 1) * EB, :] = (hs[sb] + y).astype(o_ref.dtype)
    for sb in range(nsb + 1):
        if sb < nsb:
            ffn1(sb)
        if sb >= 1:
            ffn2(sb - 1)


@jax.jit
def pallas_sequential_preLN__softmax_full_mha__dense_activation_gelu__prompt_kernel(
    A_x: jax.Array,
    A_wqkv: jax.Array,
    A_wo: jax.Array,
    B_x: jax.Array,
    B_w1: jax.Array,
    B_b1: jax.Array,
    B_w2: jax.Array,
    B_b2: jax.Array,
):
    del B_x
    B, S, D = A_x.shape
    assert B == 1
    F = B_w1.shape[1]
    BQ, CK = 512, 256
    NQ = S // BQ
    NC = S // CK
    H = _H
    Dh = D // H
    VK = CFG['VK']
    NIT = (D // 128) * (NC // CFG['CB'])
    NGRP = (128 // Dh) * CFG['CB']

    x = A_x.reshape(S, D)

    hbm = pl.BlockSpec(memory_space=pl.ANY)
    full = lambda shape: pl.BlockSpec(shape, lambda i: (0,) * len(shape))
    kern = functools.partial(_kernel, S=S, D=D, BQ=BQ, CK=CK, **CFG)
    out = pl.pallas_call(
        kern,
        grid=(NQ,),
        in_specs=[hbm] * 7,
        out_specs=pl.BlockSpec((BQ, D), lambda i: (i, 0)),
        out_shape=jax.ShapeDtypeStruct((S, D), A_x.dtype),
        scratch_shapes=[
            pltpu.VMEM((S, D), BF16),
            pltpu.VMEM((NQ, BQ, D), BF16),
            pltpu.VMEM((3, D, D), BF16),
            pltpu.VMEM((D, D), BF16),
            pltpu.VMEM((D, F), BF16),
            pltpu.VMEM((F, D), BF16),
            pltpu.VMEM((2 * D, D), BF16),
            pltpu.VMEM((D // 128, S // 2, 128), U32),
            pltpu.VMEM((D // 128, NC, VK, 128), F32),
            pltpu.VMEM((NQ, H, Dh // 2, BQ), U32),
            pltpu.VMEM((NQ, H, Dh, BQ), F32),
            pltpu.VMEM((NC, H, Dh // 2, CK), U32),
            pltpu.VMEM((NQ, H, Dh + 8, BQ), F32),
            pltpu.VMEM((NIT + 1, NGRP, Dh, VK, 128), F32),
            pltpu.VMEM((NQ, VK, BQ), F32),
            pltpu.VMEM((64, S), U32),
            pltpu.VMEM((BQ, D), BF16),
            pltpu.VMEM((F,), BF16),
            pltpu.VMEM((D,), BF16),
            pltpu.VMEM((CK, BQ), F32),
            pltpu.VMEM((NQ, H, 8, BQ), F32),
            pltpu.SemaphoreType.DMA((8 + len(CFG['XB']) - 1,)),
        ],
        compiler_params=pltpu.CompilerParams(
            dimension_semantics=("arbitrary",),
            vmem_limit_bytes=120 * 1024 * 1024),
    )(x, A_wqkv, A_wo, B_w1, B_b1, B_w2, B_b2)
    return out.reshape(B, S, D)
```

```python
import functools
import math

import jax
import jax.numpy as jnp
import jax.experimental.pallas as pl
import jax.experimental.pallas.tpu as pltpu

F32 = jnp.float32
BF16 = jnp.bfloat16
U32 = jnp.uint32

_H = 32
_EPS = 1e-5
_LOG2E = math.log2(math.e)
_SAFE_LOG2 = 60.0
_SAFE_V = 2.0 ** 40

_BQ = 512
_CK = 256
_VK = 32
_CB = 2
_RB = 128
_GATE = 2
_XL = (0, 3, 5, 7, 9, 11, 13)
_XB = (0, 512, 1536, 2048)
_WROW = 1536


def _dot(a, b):
    return jax.lax.dot_general(a, b, (((1,), (0,)), ((), ())), preferred_element_type=F32)


def _dot_nt(a, b):
    return jax.lax.dot_general(a, b, (((1,), (1,)), ((), ())), preferred_element_type=F32)


def _pack(a):
    return pltpu.bitcast(a.astype(BF16), U32)


def _unpack(a):
    return pltpu.bitcast(a, BF16)


def _fold_max(a):
    r, c = a.shape
    a = jnp.max(a.reshape(r // 8, 8, c), axis=0)
    m = a[:, 0:128]
    for t in range(1, c // 128):
        m = jnp.maximum(m, a[:, t * 128:(t + 1) * 128])
    return m


def _kernel(x_hbm, wqkv_hbm, wo_hbm, w1_hbm, b1_hbm, w2_hbm, b2_hbm, o_ref,
            x_scr, xn_scr, wqkv_scr, wo_scr, w1_scr, w2_scr, wt_scr,
            k_scr, kf_scr, qt_scr, qf_scr, vt_scr, acc_scr, kb_scr, sv_scr, wq_scr,
            b1_scr, b2_scr, pc_scr, qg_scr, sems, *, S, D):
    H, BQ, CK, VK, CB, RB = _H, _BQ, _CK, _VK, _CB, _RB
    Dh = D // H
    HG = 128 // Dh
    NG = H // HG
    NC = S // CK
    NQ = S // BQ
    CPB = BQ // CK
    NT = BQ // 128
    MK = CK - VK
    NCB = NC // CB
    NIT = NG * NCB
    NGRP = HG * CB
    NSTEP = NGRP * NQ
    A = NQ
    assert VK // 8 == NQ
    i = pl.program_id(0)

    def x_copy(j):
        rows = pl.ds(_XB[j], _XB[j + 1] - _XB[j])
        return pltpu.make_async_copy(x_hbm.at[rows], x_scr.at[rows], sems.at[8 + j])

    def w_copy(j):
        return pltpu.make_async_copy(wqkv_hbm.at[:, pl.ds(j * D, D)], wqkv_scr.at[j], sems.at[j])
    late_copies = [pltpu.make_async_copy(src, dst, sems.at[3 + n]) for n, (src, dst) in enumerate(
        [(wo_hbm, wo_scr), (w1_hbm, w1_scr), (w2_hbm, w2_scr), (b1_hbm, b1_scr), (b2_hbm, b2_scr)])]

    def vpu_scores(kb, h, qb, state, side=None):
        res = {}
        for g16 in range(VK // 16):
            for qt in range(NT):
                if side is not None:
                    side((qb * (VK // 16) + g16) * NT + qt)
                lanes = slice(qt * 128, (qt + 1) * 128)
                a = [None, None]
                for d in range(Dh):
                    qv = jnp.broadcast_to(qf_scr[qb, h, d:d + 1, lanes], (8, 128))
                    if d == _GATE and state is not None and state['tok'] is not None:
                        q2 = jnp.broadcast_to(qg_scr[qb, h, d:d + 1, lanes], (8, 128))
                        qv = jnp.where(state['tok'], qv, q2)
                    for s in range(2):
                        t = kb(d, g16 * 16 + s * 8) * qv
                        a[s] = t if a[s] is None else a[s] + t
                if state is not None:
                    state['tok'] = a[0] > a[1]
                res[(g16, qt)] = a
        rows = [jnp.concatenate([res[(g16, qt)][s] for qt in range(NT)], axis=1)
                for g16 in range(VK // 16) for s in range(2)]
        return jnp.concatenate(rows, axis=0)

    @pl.when(i == 0)
    def _attention():
        w_copy(1).start()
        for j in range(len(_XB) - 1):
            x_copy(j).start()
        w_copy(0).start()
        w_copy(2).start()
        for cp in late_copies:
            cp.start()
        acc_scr[...] = jnp.zeros(acc_scr.shape, F32)
        pc_scr[...] = jnp.zeros(pc_scr.shape, F32)

        w_copy(1).wait()
        wk_cs = _dot(jnp.ones((8, D), BF16), wqkv_scr[1])[0:1]
        kk_max = None
        for t0 in range(0, S, RB):
            if t0 in _XB:
                x_copy(_XB.index(t0)).wait()
            if t0 == _WROW:
                w_copy(0).wait()
                w_copy(2).wait()
                wt_scr[0:D, :] = wqkv_scr[0].T
                wt_scr[D:2 * D, :] = wqkv_scr[2].T
            xb = x_scr[t0:t0 + RB, :]
            xf = xb.astype(F32)
            m = jnp.mean(xf, axis=-1, keepdims=True)
            xc = xf - m
            r = jax.lax.rsqrt(jnp.mean(xc * xc, axis=-1, keepdims=True) + _EPS)
            xn_scr[t0 // BQ, t0 % BQ:t0 % BQ + RB, :] = (xc * r).astype(BF16)
            kf = (_dot(xb, wqkv_scr[1]) - m * wk_cs) * r
            for g in range(NG):
                k_scr[g, t0 // 2:(t0 + RB) // 2, :] = _pack(kf[:, g * 128:(g + 1) * 128])
                for c in range(NC):
                    lo, hi = c * CK + MK - t0, (c + 1) * CK - t0
                    if lo >= 0 and hi <= RB:
                        kf_scr[g, c] = kf[lo:hi, g * 128:(g + 1) * 128].astype(BF16).astype(F32)
            kk = jnp.max((kf * kf).reshape(RB // 64, 64, D), axis=0)
            kk_max = kk if kk_max is None else jnp.maximum(kk_max, kk)
        for d in range(Dh):
            kb_scr[NIT, 0, d] = jnp.broadcast_to(kf_scr[0, 0][:, d:d + 1], (VK, 128))
        seg = (jax.lax.broadcasted_iota(jnp.int32, (D, 128), 0) // Dh
               == jax.lax.broadcasted_iota(jnp.int32, (D, 128), 1)).astype(BF16)
        kn_max = jnp.max(_dot((kk_max * 1.03).astype(BF16), seg))

        qscale = (Dh ** -0.5) * _LOG2E

        def proj(tb, carry):
            qn_max, v_max = carry
            qv = _dot_nt(wt_scr[...], xn_scr[tb])
            qf = (qv[0:D] * qscale).astype(BF16).astype(F32)
            qt_scr[tb] = _pack(qf).reshape(H, Dh // 2, BQ)
            qf_scr[tb] = qf.reshape(H, Dh, BQ)
            qg_scr[tb] = qf.reshape(H, Dh, BQ)[:, 0:8, :]
            for cc in range(CPB):
                vt_scr[tb * CPB + cc] = _pack(qv[D:2 * D, cc * CK:(cc + 1) * CK]).reshape(H, Dh // 2, CK)
            qn_max = jnp.maximum(qn_max, _fold_max(jnp.sum((qf * qf).reshape(H, Dh, BQ), axis=1)))
            v_max = jnp.maximum(v_max, _fold_max(jnp.abs(qv[D:2 * D])))
            sv_scr[tb] = vpu_scores(lambda d, r: kb_scr[NIT, 0, d, r:r + 8, :], 0, tb, None)
            r8 = pl.multiple_of(tb * 8, 8)
            for grp in range(1, NGRP + 1):
                c, hh = (grp % CB, grp // CB) if grp < NGRP else (CB, 0)
                kv = kf_scr[0, c, pl.ds(r8, 8), :]
                for d in range(Dh):
                    lane = hh * Dh + d
                    kb_scr[0, grp - 1, d, pl.ds(r8, 8), :] = jnp.broadcast_to(kv[:, lane:lane + 1], (8, 128))
            return qn_max, v_max

        qn_max, v_max = jax.lax.fori_loop(
            0, NQ, proj, (jnp.zeros((8, 128), F32), jnp.zeros((8, 128), F32)), unroll=NQ)
        bound2 = jnp.max(qn_max) * kn_max
        fast = jnp.logical_and(bound2 <= _SAFE_LOG2 * _SAFE_LOG2, jnp.max(v_max) <= _SAFE_V)

        def pv_carry(t):
            h = (t // NCB) * HG + HG - 1
            c = (t % NCB) * CB + CB - 1
            o = _dot(_unpack(vt_scr[c, h]), pc_scr[...])
            acc_scr[NQ - 1, h, 0:Dh, :] = o + acc_scr[NQ - 1, h, 0:Dh, :]

        @pl.when(fast)
        def _fast():
            def body(it, carry):
                its = [it, jnp.minimum(it + 1, NIT - 1), jnp.minimum(it + 2, NIT - 1)]
                gs = [t // NCB for t in its]
                cs = [(t % NCB) * CB for t in its]
                g, c0 = gs[0], cs[0]
                seq = [(hh, cc, qb) for hh in range(HG) for cc in range(CB) for qb in range(NQ)]
                state = dict(tok=None, xtok=None)
                sv, pts, part, lsum = {}, {}, {}, {}

                def group(grp):
                    b, r = grp // NGRP, grp % NGRP
                    return gs[b], cs[b] + r % CB, r // CB

                def vpu(j):
                    grp, qb = j // NQ, j % NQ
                    gg, _, hh = group(grp)

                    def side(idx):
                        if idx % 2:
                            return
                        d = idx // 2
                        gb, cb, hb = group(grp + NGRP)
                        lane = hb * Dh + d
                        kv = kf_scr[gb, cb]
                        if d in _XL and state['xtok'] is not None:
                            kv = jnp.concatenate([kv[0:8] + state['xtok'], kv[8:]], axis=0)
                        v = jnp.broadcast_to(kv[:, lane:lane + 1], (VK, 128))
                        kb_scr[it + 1, grp - 1, d] = v
                        if d in _XL:
                            w = v[0:8]
                            state['xtok'] = w - w
                    r = vpu_scores(lambda d, r: kb_scr[it, grp - 1, d, r:r + 8, :],
                                   gg * HG + hh, qb, state, side)
                    if j >= NSTEP:
                        sv_scr[j - NSTEP] = r
                    else:
                        sv[j] = r

                def qk(j):
                    hh, cc, qb = seq[j]
                    parts = []
                    if hh > 0:
                        parts.append(jnp.zeros((hh * Dh, BQ), BF16))
                    parts.append(_unpack(qt_scr[qb, g * HG + hh]))
                    if hh < HG - 1:
                        parts.append(jnp.zeros(((HG - 1 - hh) * Dh, BQ), BF16))
                    wq = jnp.concatenate(parts, axis=0)
                    r0 = pl.multiple_of((c0 + cc) * (CK // 2), CK // 2)
                    r = sv_scr[j] if j < A else sv.pop(j)
                    st = _dot(_unpack(k_scr[g, pl.ds(r0, MK // 2), :]), wq)
                    p = jnp.exp2(jnp.concatenate([st, r], axis=0))
                    ps = jnp.sum(p.reshape(CK // 8, 8, BQ), axis=0)
                    lsum[(hh, qb)] = ps if cc == 0 else ps + lsum[(hh, qb)]
                    pts[j] = p

                def pv(j):
                    hh, cc, qb = seq[j]
                    h = g * HG + hh
                    last = (hh, qb) == (HG - 1, NQ - 1)
                    o = _dot(_unpack(vt_scr[c0 + cc, h]), pts.pop(j))
                    if cc == 0:
                        part[(hh, qb)] = o + acc_scr[qb, h, 0:Dh, :]
                    else:
                        part[(hh, qb)] = o + part[(hh, qb)]
                    if cc == CB - 1 - (1 if last else 0):
                        acc_scr[qb, h, 0:Dh, :] = part.pop((hh, qb))
                    if cc == CB - 1:
                        acc_scr[qb, h, Dh:Dh + 8, :] = lsum.pop((hh, qb)) + acc_scr[qb, h, Dh:Dh + 8, :]

                for j in range(NSTEP + 1):
                    if j < NSTEP:
                        qk(j)
                        vpu(j + A)
                    if j == 0:
                        pv_carry(jnp.maximum(it - 1, 0))
                    elif j == NSTEP:
                        pc_scr[...] = pts.pop(j - 1)
                        h = g * HG + HG - 1
                        acc_scr[NQ - 1, h, Dh:Dh + 8, :] = (lsum.pop((HG - 1, NQ - 1))
                                                            + acc_scr[NQ - 1, h, Dh:Dh + 8, :])
                    else:
                        pv(j - 1)
                return carry
            jax.lax.fori_loop(0, NIT, body, 0)
            pv_carry(NIT - 1)
            v = kb_scr[NIT, 0, 0, 0:8, :]
            acc_scr[0, 0, Dh:Dh + 8, 0:128] = acc_scr[0, 0, Dh:Dh + 8, 0:128] + (v - v)

        @pl.when(jnp.logical_not(fast))
        def _slow():
            def head(h, carry):
                g = h // HG
                wq_scr[...] = jnp.zeros(wq_scr.shape, U32)
                r0 = pl.multiple_of((h % HG) * (Dh // 2), Dh // 2)
                for qb in range(NQ):
                    wq_scr[pl.ds(r0, Dh // 2), qb * BQ:(qb + 1) * BQ] = qt_scr[qb, h]

                def scores(c):
                    kc = k_scr[g, pl.ds(pl.multiple_of(c * (CK // 2), CK // 2), CK // 2), :]
                    return _dot(_unpack(kc), _unpack(wq_scr[...]))

                def mx(c, m):
                    return jnp.maximum(m, jnp.max(scores(c).reshape(CK // 8, 8, S), axis=0))
                m8 = jax.lax.fori_loop(0, NC, mx, jnp.full((8, S), -jnp.inf, F32))
                m = jnp.max(m8, axis=0, keepdims=True)

                def acc(c, carry):
                    o, l = carry
                    p = jnp.exp2(scores(c) - m)
                    return (o + _dot(_unpack(vt_scr[c, h]), p.astype(BF16)),
                            l + jnp.sum(p.reshape(CK // 8, 8, S), axis=0))
                o, l = jax.lax.fori_loop(0, NC, acc, (jnp.zeros((Dh, S), F32), jnp.zeros((8, S), F32)))
                for qb in range(NQ):
                    acc_scr[qb, h, 0:Dh, :] = o[:, qb * BQ:(qb + 1) * BQ]
                    acc_scr[qb, h, Dh:Dh + 8, :] = l[:, qb * BQ:(qb + 1) * BQ]
                return carry
            jax.lax.fori_loop(0, H, head, 0)

        for cp in late_copies:
            cp.wait()

    a = acc_scr[i]
    l = jnp.sum(a[:, Dh:Dh + 8, :], axis=1, keepdims=True)
    inv = pl.reciprocal(l, approx=True)
    inv = inv * (2.0 - l * inv)
    o = (a[:, 0:Dh, :] * inv).reshape(D, BQ).T.astype(BF16)
    b1 = b1_scr[...].astype(F32)[None, :]
    b2 = b2_scr[...].astype(F32)[None, :]
    r0 = pl.multiple_of(i * BQ, BQ)
    h = x_scr[pl.ds(r0, BQ), :].astype(F32) + _dot(o, wo_scr[...])
    hc = h - jnp.mean(h, axis=-1, keepdims=True)
    r = jax.lax.rsqrt(jnp.mean(hc * hc, axis=-1, keepdims=True) + _EPS)
    z = _dot(hc.astype(BF16), w1_scr[...]) * r + b1
    gl = jax.nn.gelu(z, approximate=True).astype(BF16)
    y = _dot(gl, w2_scr[...]) + b2
    o_ref[...] = (h + y).astype(o_ref.dtype)


@jax.jit
def pallas_sequential_preLN__softmax_full_mha__dense_activation_gelu__prompt_kernel(
    A_x: jax.Array,
    A_wqkv: jax.Array,
    A_wo: jax.Array,
    B_x: jax.Array,
    B_w1: jax.Array,
    B_b1: jax.Array,
    B_w2: jax.Array,
    B_b2: jax.Array,
):
    del B_x
    B, S, D = A_x.shape
    assert B == 1 and S == _XB[-1]
    F = B_w1.shape[1]
    H, BQ, CK, VK = _H, _BQ, _CK, _VK
    Dh = D // H
    NQ = S // BQ
    NC = S // CK
    NIT = (D // 128) * (NC // _CB)
    NGRP = (128 // Dh) * _CB

    out = pl.pallas_call(
        functools.partial(_kernel, S=S, D=D),
        grid=(NQ,),
        in_specs=[pl.BlockSpec(memory_space=pl.ANY)] * 7,
        out_specs=pl.BlockSpec((BQ, D), lambda i: (i, 0)),
        out_shape=jax.ShapeDtypeStruct((S, D), A_x.dtype),
        scratch_shapes=[
            pltpu.VMEM((S, D), BF16),
            pltpu.VMEM((NQ, BQ, D), BF16),
            pltpu.VMEM((3, D, D), BF16),
            pltpu.VMEM((D, D), BF16),
            pltpu.VMEM((D, F), BF16),
            pltpu.VMEM((F, D), BF16),
            pltpu.VMEM((2 * D, D), BF16),
            pltpu.VMEM((D // 128, S // 2, 128), U32),
            pltpu.VMEM((D // 128, NC, VK, 128), F32),
            pltpu.VMEM((NQ, H, Dh // 2, BQ), U32),
            pltpu.VMEM((NQ, H, Dh, BQ), F32),
            pltpu.VMEM((NC, H, Dh // 2, CK), U32),
            pltpu.VMEM((NQ, H, Dh + 8, BQ), F32),
            pltpu.VMEM((NIT + 1, NGRP, Dh, VK, 128), F32),
            pltpu.VMEM((NQ, VK, BQ), F32),
            pltpu.VMEM((64, S), U32),
            pltpu.VMEM((F,), BF16),
            pltpu.VMEM((D,), BF16),
            pltpu.VMEM((CK, BQ), F32),
            pltpu.VMEM((NQ, H, 8, BQ), F32),
            pltpu.SemaphoreType.DMA((8 + len(_XB) - 1,)),
        ],
        compiler_params=pltpu.CompilerParams(
            dimension_semantics=("arbitrary",),
            vmem_limit_bytes=120 * 1024 * 1024),
    )(A_x.reshape(S, D), A_wqkv, A_wo, B_w1, B_b1, B_w2, B_b2)
    return out.reshape(B, S, D)
```

```python
import functools
import math

import jax
import jax.numpy as jnp
import jax.experimental.pallas as pl
import jax.experimental.pallas.tpu as pltpu

F32 = jnp.float32
BF16 = jnp.bfloat16
U32 = jnp.uint32

_H = 32
_EPS = 1e-5
_LOG2E = math.log2(math.e)
_SAFE_LOG2 = 60.0
_SAFE_V = 2.0 ** 40

_BIG = 2.0 ** 100

_BQ = 512
_CK = 256
_VK = 32
_CB = 2
_RB = 128
_GATE = 2
_XL = (0, 3, 5, 7, 9, 11, 13)
_XB = (0, 512, 1536, 2048)
_WROW = 1536


def _dot(a, b):
    return jax.lax.dot_general(a, b, (((1,), (0,)), ((), ())), preferred_element_type=F32)


def _dot_nt(a, b):
    return jax.lax.dot_general(a, b, (((1,), (1,)), ((), ())), preferred_element_type=F32)


def _pack(a):
    return pltpu.bitcast(a.astype(BF16), U32)


def _unpack(a):
    return pltpu.bitcast(a, BF16)


def _fold_max(a):
    r, c = a.shape
    a = jnp.max(a.reshape(r // 8, 8, c), axis=0)
    m = a[:, 0:128]
    for t in range(1, c // 128):
        m = jnp.maximum(m, a[:, t * 128:(t + 1) * 128])
    return m


def _kernel(x_hbm, wqkv_hbm, wo_hbm, w1_hbm, b1_hbm, w2_hbm, b2_hbm, o_ref,
            x_scr, xn_scr, wqkv_scr, wo_scr, w1_scr, w2_scr, wt_scr,
            k_scr, kf_scr, qt_scr, qf_scr, vt_scr, acc_scr, kb_scr, sv_scr, wq_scr,
            b1_scr, b2_scr, pc_scr, qg_scr, wot_scr, sems, *, S, D):
    H, BQ, CK, VK, CB, RB = _H, _BQ, _CK, _VK, _CB, _RB
    Dh = D // H
    HG = 128 // Dh
    NG = H // HG
    NC = S // CK
    NQ = S // BQ
    CPB = BQ // CK
    NT = BQ // 128
    MK = CK - VK
    NCB = NC // CB
    NIT = NG * NCB
    NGRP = HG * CB
    NSTEP = NGRP * NQ
    A = NQ
    assert CB == 2 and D == NQ * 128
    i = pl.program_id(0)

    def x_copy(j):
        rows = pl.ds(_XB[j], _XB[j + 1] - _XB[j])
        return pltpu.make_async_copy(x_hbm.at[rows], x_scr.at[rows], sems.at[8 + j])

    def w_copy(j):
        return pltpu.make_async_copy(wqkv_hbm.at[:, pl.ds(j * D, D)], wqkv_scr.at[j], sems.at[j])
    late_copies = [pltpu.make_async_copy(src, dst, sems.at[3 + n]) for n, (src, dst) in enumerate(
        [(wo_hbm, wo_scr), (w1_hbm, w1_scr), (w2_hbm, w2_scr), (b1_hbm, b1_scr), (b2_hbm, b2_scr)])]

    def vpu_scores(kb, h, qb, state, side):
        res = {}
        for g16 in range(VK // 16):
            for qt in range(NT):
                side((qb * (VK // 16) + g16) * NT + qt)
                lanes = slice(qt * 128, (qt + 1) * 128)
                a = [None, None]
                for d in range(Dh):
                    qv = jnp.broadcast_to(qf_scr[qb, h, d:d + 1, lanes], (8, 128))
                    if d == _GATE and state['tok'] is not None:
                        q2 = jnp.broadcast_to(qg_scr[qb, h, d:d + 1, lanes], (8, 128))
                        qv = jnp.where(state['tok'], qv, q2)
                    for s in range(2):
                        t = kb(d, g16 * 16 + s * 8) * qv
                        a[s] = t if a[s] is None else a[s] + t
                state['tok'] = a[0] > a[1]
                res[(g16, qt)] = a
        rows = [jnp.concatenate([res[(g16, qt)][s] for qt in range(NT)], axis=1)
                for g16 in range(VK // 16) for s in range(2)]
        return jnp.concatenate(rows, axis=0)

    @pl.when(i == 0)
    def _attention():
        w_copy(1).start()
        for j in range(len(_XB) - 1):
            x_copy(j).start()
        w_copy(0).start()
        w_copy(2).start()
        for cp in late_copies:
            cp.start()
        acc_scr[...] = jnp.zeros(acc_scr.shape, F32)
        pc_scr[...] = jnp.zeros(pc_scr.shape, F32)

        w_copy(1).wait()
        wk_cs = _dot(jnp.ones((8, D), BF16), wqkv_scr[1])[0:1]
        kk_max = None
        for t0 in range(0, S, RB):
            if t0 in _XB:
                x_copy(_XB.index(t0)).wait()
            if t0 == _WROW:
                w_copy(0).wait()
                w_copy(2).wait()
                late_copies[0].wait()
                wt_scr[0:D, :] = wqkv_scr[0].T
                wt_scr[D:2 * D, :] = wqkv_scr[2].T
            xb = x_scr[t0:t0 + RB, :]
            xf = xb.astype(F32)
            m = jnp.mean(xf, axis=-1, keepdims=True)
            xc = xf - m
            r = jax.lax.rsqrt(jnp.mean(xc * xc, axis=-1, keepdims=True) + _EPS)
            xn_scr[t0 // BQ, t0 % BQ:t0 % BQ + RB, :] = (xc * r).astype(BF16)
            kf = (_dot(xb, wqkv_scr[1]) - m * wk_cs) * r
            for g in range(NG):
                k_scr[g, t0 // 2:(t0 + RB) // 2, :] = _pack(kf[:, g * 128:(g + 1) * 128])
                for c in range(NC):
                    lo, hi = c * CK + MK - t0, (c + 1) * CK - t0
                    if lo >= 0 and hi <= RB:
                        kf_scr[g, c] = kf[lo:hi, g * 128:(g + 1) * 128].astype(BF16).astype(F32)
            kk = jnp.max((kf * kf).reshape(RB // 64, 64, D), axis=0)
            kk_max = kk if kk_max is None else jnp.maximum(kk_max, kk)

        def kn_bound():
            seg = (jax.lax.broadcasted_iota(jnp.int32, (D, 128), 0) // Dh
                   == jax.lax.broadcasted_iota(jnp.int32, (D, 128), 1)).astype(BF16)
            return jnp.max(_dot(jnp.minimum(kk_max * 1.03, _BIG).astype(BF16), seg))

        qscale = (Dh ** -0.5) * _LOG2E

        def proj(tb, carry):
            qn_max, v_max = carry
            qv = _dot_nt(wt_scr[...], xn_scr[tb])
            qf = (qv[0:D] * qscale).astype(BF16).astype(F32)
            qt_scr[tb] = _pack(qf).reshape(H, Dh // 2, BQ)
            qf_scr[tb] = qf.reshape(H, Dh, BQ)
            qg_scr[tb] = qf.reshape(H, Dh, BQ)[:, 0:8, :]
            for cc in range(CPB):
                vt_scr[tb * CPB + cc] = _pack(qv[D:2 * D, cc * CK:(cc + 1) * CK]).reshape(H, Dh // 2, CK)
            qn_max = jnp.maximum(qn_max, _fold_max(jnp.sum((qf * qf).reshape(H, Dh, BQ), axis=1)))
            v_max = jnp.maximum(v_max, _fold_max(jnp.abs(qv[D:2 * D])))
            wot_scr[tb] = wo_scr[tb * 128:(tb + 1) * 128, :].T
            for hh in range(tb * HG // NQ, (tb + 1) * HG // NQ):
                grps = [(2 * hh + 1, 1), (2 * hh, 0) if hh else (NGRP, CB)]
                kv = jnp.concatenate([kf_scr[0, c] for _, c in grps], axis=0)
                for d in range(Dh):
                    lane = hh * Dh + d
                    v = jnp.broadcast_to(kv[:, lane:lane + 1], (2 * VK, 128))
                    for n, (grp, _) in enumerate(grps):
                        kb_scr[0, grp - 1, d] = v[n * VK:(n + 1) * VK]
            return qn_max, v_max

        qn_max, v_max = jnp.zeros((8, 128), F32), jnp.zeros((8, 128), F32)
        for tb in range(NQ):
            qn_max, v_max = proj(tb, (qn_max, v_max))
            if tb == NQ - 2:
                kn_max = kn_bound()
        for tb in range(NQ):
            wq0 = jnp.concatenate([_unpack(qt_scr[tb, 0]), jnp.zeros((128 - Dh, BQ), BF16)], axis=0)
            sv_scr[tb] = _dot(_unpack(k_scr[0, MK // 2:CK // 2, :]), wq0)
        bound2 = jnp.max(qn_max) * kn_max
        fast = jnp.logical_and(jnp.logical_and(bound2 <= _SAFE_LOG2 * _SAFE_LOG2, kn_max < 0.5 * _BIG),
                               jnp.max(v_max) <= _SAFE_V)

        def pv_carry(t):
            h = (t // NCB) * HG + HG - 1
            c = (t % NCB) * CB + CB - 1
            o = _dot(_unpack(vt_scr[c, h]), pc_scr[...])
            acc_scr[NQ - 1, h, 0:Dh, :] = o + acc_scr[NQ - 1, h, 0:Dh, :]

        @pl.when(fast)
        def _fast():
            def body(it, carry):
                its = [it, jnp.minimum(it + 1, NIT - 1), jnp.minimum(it + 2, NIT - 1)]
                gs = [t // NCB for t in its]
                cs = [(t % NCB) * CB for t in its]
                g, c0 = gs[0], cs[0]
                seq = [(hh, cc, qb) for hh in range(HG) for cc in range(CB) for qb in range(NQ)]
                state = dict(tok=None, xtok=None)
                sv, pts, part, lsum = {}, {}, {}, {}

                def group(grp):
                    b, r = grp // NGRP, grp % NGRP
                    return gs[b], cs[b] + r % CB, r // CB

                def vpu(j):
                    grp, qb = j // NQ, j % NQ
                    gg, _, hh = group(grp)

                    def side(idx):
                        if idx % 2:
                            return
                        d = idx // 2
                        gb, cb, hb = group(grp + NGRP)
                        lane = hb * Dh + d
                        kv = kf_scr[gb, cb]
                        if d in _XL and state['xtok'] is not None:
                            kv = jnp.concatenate([kv[0:8] + state['xtok'], kv[8:]], axis=0)
                        v = jnp.broadcast_to(kv[:, lane:lane + 1], (VK, 128))
                        kb_scr[it + 1, grp - 1, d] = v
                        if d in _XL:
                            w = v[0:8]
                            state['xtok'] = w - w
                    r = vpu_scores(lambda d, r: kb_scr[it, grp - 1, d, r:r + 8, :],
                                   gg * HG + hh, qb, state, side)
                    if j >= NSTEP:
                        sv_scr[j - NSTEP] = r
                    else:
                        sv[j] = r

                def qk(j):
                    hh, cc, qb = seq[j]
                    parts = []
                    if hh > 0:
                        parts.append(jnp.zeros((hh * Dh, BQ), BF16))
                    parts.append(_unpack(qt_scr[qb, g * HG + hh]))
                    if hh < HG - 1:
                        parts.append(jnp.zeros(((HG - 1 - hh) * Dh, BQ), BF16))
                    wq = jnp.concatenate(parts, axis=0)
                    r0 = pl.multiple_of((c0 + cc) * (CK // 2), CK // 2)
                    r = sv_scr[j] if j < A else sv.pop(j)
                    st = _dot(_unpack(k_scr[g, pl.ds(r0, MK // 2), :]), wq)
                    p = jnp.exp2(jnp.concatenate([st, r], axis=0))
                    ps = jnp.sum(p.reshape(CK // 8, 8, BQ), axis=0)
                    lsum[(hh, qb)] = ps if cc == 0 else ps + lsum[(hh, qb)]
                    pts[j] = p

                def pv(j):
                    hh, cc, qb = seq[j]
                    h = g * HG + hh
                    last = (hh, qb) == (HG - 1, NQ - 1)
                    o = _dot(_unpack(vt_scr[c0 + cc, h]), pts.pop(j))
                    if cc == 0:
                        part[(hh, qb)] = o + acc_scr[qb, h, 0:Dh, :]
                    else:
                        part[(hh, qb)] = o + part[(hh, qb)]
                    if cc == CB - 1 - (1 if last else 0):
                        acc_scr[qb, h, 0:Dh, :] = part.pop((hh, qb))
                    if cc == CB - 1:
                        acc_scr[qb, h, Dh:Dh + 8, :] = lsum.pop((hh, qb)) + acc_scr[qb, h, Dh:Dh + 8, :]

                for j in range(NSTEP + 1):
                    if j < NSTEP:
                        qk(j)
                        vpu(j + A)
                    if j == 0:
                        pv_carry(jnp.maximum(it - 1, 0))
                    elif j == NSTEP:
                        pc_scr[...] = pts.pop(j - 1)
                        h = g * HG + HG - 1
                        acc_scr[NQ - 1, h, Dh:Dh + 8, :] = (lsum.pop((HG - 1, NQ - 1))
                                                            + acc_scr[NQ - 1, h, Dh:Dh + 8, :])
                    else:
                        pv(j - 1)
                return carry
            jax.lax.fori_loop(0, NIT, body, 0)
            pv_carry(NIT - 1)
            v = kb_scr[NIT, 0, 0, 0:8, :]
            acc_scr[0, 0, Dh:Dh + 8, 0:128] = acc_scr[0, 0, Dh:Dh + 8, 0:128] + (v - v)

        @pl.when(jnp.logical_not(fast))
        def _slow():
            def head(h, carry):
                g = h // HG
                wq_scr[...] = jnp.zeros(wq_scr.shape, U32)
                r0 = pl.multiple_of((h % HG) * (Dh // 2), Dh // 2)
                for qb in range(NQ):
                    wq_scr[pl.ds(r0, Dh // 2), qb * BQ:(qb + 1) * BQ] = qt_scr[qb, h]

                def scores(c):
                    kc = k_scr[g, pl.ds(pl.multiple_of(c * (CK // 2), CK // 2), CK // 2), :]
                    return _dot(_unpack(kc), _unpack(wq_scr[...]))

                def mx(c, m):
                    return jnp.maximum(m, jnp.max(scores(c).reshape(CK // 8, 8, S), axis=0))
                m8 = jax.lax.fori_loop(0, NC, mx, jnp.full((8, S), -jnp.inf, F32))
                m = jnp.max(m8, axis=0, keepdims=True)

                def acc(c, carry):
                    o, l = carry
                    p = jnp.exp2(scores(c) - m)
                    return (o + _dot(_unpack(vt_scr[c, h]), p.astype(BF16)),
                            l + jnp.sum(p.reshape(CK // 8, 8, S), axis=0))
                o, l = jax.lax.fori_loop(0, NC, acc, (jnp.zeros((Dh, S), F32), jnp.zeros((8, S), F32)))
                for qb in range(NQ):
                    acc_scr[qb, h, 0:Dh, :] = o[:, qb * BQ:(qb + 1) * BQ]
                    acc_scr[qb, h, Dh:Dh + 8, :] = l[:, qb * BQ:(qb + 1) * BQ]
                return carry
            jax.lax.fori_loop(0, H, head, 0)

        for cp in late_copies[1:]:
            cp.wait()

    a = acc_scr[i]
    l = jnp.sum(a[:, Dh:Dh + 8, :], axis=1, keepdims=True)
    inv = pl.reciprocal(l, approx=True)
    inv = inv * (2.0 - l * inv)
    ot = (a[:, 0:Dh, :] * inv).reshape(D, BQ)
    b1 = b1_scr[...].astype(F32)[None, :]
    b2 = b2_scr[...].astype(F32)[None, :]
    r0 = pl.multiple_of(i * BQ, BQ)
    ao = _dot(jnp.concatenate([wot_scr[t] for t in range(NQ)], axis=1), ot).T
    h = x_scr[pl.ds(r0, BQ), :].astype(F32) + ao
    hc = h - jnp.mean(h, axis=-1, keepdims=True)
    r = jax.lax.rsqrt(jnp.mean(hc * hc, axis=-1, keepdims=True) + _EPS)
    z = _dot(hc.astype(BF16), w1_scr[...]) * r + b1
    gl = jax.nn.gelu(z, approximate=True).astype(BF16)
    y = _dot(gl, w2_scr[...]) + b2
    o_ref[...] = (h + y).astype(o_ref.dtype)


@jax.jit
def pallas_sequential_preLN__softmax_full_mha__dense_activation_gelu__prompt_kernel(
    A_x: jax.Array,
    A_wqkv: jax.Array,
    A_wo: jax.Array,
    B_x: jax.Array,
    B_w1: jax.Array,
    B_b1: jax.Array,
    B_w2: jax.Array,
    B_b2: jax.Array,
):
    del B_x
    B, S, D = A_x.shape
    assert B == 1 and S == _XB[-1]
    F = B_w1.shape[1]
    H, BQ, CK, VK = _H, _BQ, _CK, _VK
    Dh = D // H
    NQ = S // BQ
    NC = S // CK
    NIT = (D // 128) * (NC // _CB)
    NGRP = (128 // Dh) * _CB

    out = pl.pallas_call(
        functools.partial(_kernel, S=S, D=D),
        grid=(NQ,),
        in_specs=[pl.BlockSpec(memory_space=pl.ANY)] * 7,
        out_specs=pl.BlockSpec((BQ, D), lambda i: (i, 0)),
        out_shape=jax.ShapeDtypeStruct((S, D), A_x.dtype),
        scratch_shapes=[
            pltpu.VMEM((S, D), BF16),
            pltpu.VMEM((NQ, BQ, D), BF16),
            pltpu.VMEM((3, D, D), BF16),
            pltpu.VMEM((D, D), BF16),
            pltpu.VMEM((D, F), BF16),
            pltpu.VMEM((F, D), BF16),
            pltpu.VMEM((2 * D, D), BF16),
            pltpu.VMEM((D // 128, S // 2, 128), U32),
            pltpu.VMEM((D // 128, NC, VK, 128), F32),
            pltpu.VMEM((NQ, H, Dh // 2, BQ), U32),
            pltpu.VMEM((NQ, H, Dh, BQ), F32),
            pltpu.VMEM((NC, H, Dh // 2, CK), U32),
            pltpu.VMEM((NQ, H, Dh + 8, BQ), F32),
            pltpu.VMEM((NIT + 1, NGRP, Dh, VK, 128), F32),
            pltpu.VMEM((NQ, VK, BQ), F32),
            pltpu.VMEM((64, S), U32),
            pltpu.VMEM((F,), BF16),
            pltpu.VMEM((D,), BF16),
            pltpu.VMEM((CK, BQ), F32),
            pltpu.VMEM((NQ, H, 8, BQ), F32),
            pltpu.VMEM((NQ, D, 128), BF16),
            pltpu.SemaphoreType.DMA((8 + len(_XB) - 1,)),
        ],
        compiler_params=pltpu.CompilerParams(
            dimension_semantics=("arbitrary",),
            vmem_limit_bytes=120 * 1024 * 1024),
    )(A_x.reshape(S, D), A_wqkv, A_wo, B_w1, B_b1, B_w2, B_b2)
    return out.reshape(B, S, D)
```

```python
import functools
import math

import jax
import jax.numpy as jnp
import jax.experimental.pallas as pl
import jax.experimental.pallas.tpu as pltpu

F32 = jnp.float32
BF16 = jnp.bfloat16
U32 = jnp.uint32

_H = 32
_EPS = 1e-5
_LOG2E = math.log2(math.e)
_SAFE_LOG2 = 60.0
_SAFE_V = 2.0 ** 40

_BIG = 2.0 ** 100

_BQ = 512
_CK = 256
_VK = 32
_CB = 2
_RB = 128
_GATE = 2
_XL = (1, 2, 3, 4, 6, 7, 11, 12, 13)
_XB = (0, 256, 768, 1664, 2048)
_WROW = 1664


def _dot(a, b):
    return jax.lax.dot_general(a, b, (((1,), (0,)), ((), ())), preferred_element_type=F32)


def _dot_nt(a, b):
    return jax.lax.dot_general(a, b, (((1,), (1,)), ((), ())), preferred_element_type=F32)


def _pack(a):
    return pltpu.bitcast(a.astype(BF16), U32)


def _unpack(a):
    return pltpu.bitcast(a, BF16)


def _fold_max(a):
    r, c = a.shape
    a = jnp.max(a.reshape(r // 8, 8, c), axis=0)
    m = a[:, 0:128]
    for t in range(1, c // 128):
        m = jnp.maximum(m, a[:, t * 128:(t + 1) * 128])
    return m


def _kernel(x_hbm, wqkv_hbm, wo_hbm, w1_hbm, b1_hbm, w2_hbm, b2_hbm, o_ref,
            x_scr, xn_scr, wqkv_scr, wo_scr, w1_scr, w2_scr, wt_scr,
            k_scr, kf_scr, qt_scr, qf_scr, vt_scr, acc_scr, kb_scr, sv_scr, wq_scr,
            b1_scr, b2_scr, pc_scr, qg_scr, wot_scr, sems, *, S, D):
    H, BQ, CK, VK, CB, RB = _H, _BQ, _CK, _VK, _CB, _RB
    Dh = D // H
    HG = 128 // Dh
    NG = H // HG
    NC = S // CK
    NQ = S // BQ
    CPB = BQ // CK
    NT = BQ // 128
    MK = CK - VK
    NCB = NC // CB
    NIT = NG * NCB
    NGRP = HG * CB
    NSTEP = NGRP * NQ
    A = NQ
    assert CB == 2 and D == NQ * 128
    i = pl.program_id(0)

    def x_copy(j):
        rows = pl.ds(_XB[j], _XB[j + 1] - _XB[j])
        return pltpu.make_async_copy(x_hbm.at[rows], x_scr.at[rows], sems.at[8 + j])

    def w_copy(j):
        return pltpu.make_async_copy(wqkv_hbm.at[:, pl.ds(j * D, D)], wqkv_scr.at[j], sems.at[j])
    late_copies = [pltpu.make_async_copy(src, dst, sems.at[3 + n]) for n, (src, dst) in enumerate(
        [(wo_hbm, wo_scr), (w1_hbm, w1_scr), (w2_hbm, w2_scr), (b1_hbm, b1_scr), (b2_hbm, b2_scr)])]

    def vpu_scores(kb, h, qb, state, side):
        rows = []
        for g16 in range(VK // 16):
            cols = []
            for qt in range(NT):
                side((qb * (VK // 16) + g16) * NT + qt)
                lanes = slice(qt * 128, (qt + 1) * 128)
                a = None
                for d in range(Dh):
                    qv = qf_scr[qb, h, d:d + 1, lanes]
                    if d == _GATE and state['tok'] is not None:
                        q8 = jnp.where(state['tok'], jnp.broadcast_to(qv, (8, 128)),
                                       jnp.broadcast_to(qg_scr[qb, h, d:d + 1, lanes], (8, 128)))
                        qv = jnp.concatenate([q8, q8], axis=0)
                    t = kb(d, g16 * 16) * qv
                    a = t if a is None else a + t
                state['tok'] = a[0:8] > a[8:16]
                cols.append(a)
            rows.append(jnp.concatenate(cols, axis=1))
        return jnp.concatenate(rows, axis=0)

    @pl.when(i == 0)
    def _attention():
        w_copy(1).start()
        for j in range(len(_XB) - 1):
            x_copy(j).start()
        w_copy(0).start()
        w_copy(2).start()
        for cp in late_copies:
            cp.start()
        acc_scr[...] = jnp.zeros(acc_scr.shape, F32)
        pc_scr[...] = jnp.zeros(pc_scr.shape, F32)

        w_copy(1).wait()
        wk_cs = _dot(jnp.ones((8, D), BF16), wqkv_scr[1])[0:1]
        kk_max = None
        for t0 in range(0, S, RB):
            if t0 in _XB:
                x_copy(_XB.index(t0)).wait()
            if t0 == _WROW:
                w_copy(0).wait()
                w_copy(2).wait()
                late_copies[0].wait()
                wt_scr[0:D, :] = wqkv_scr[0].T
                wt_scr[D:2 * D, :] = wqkv_scr[2].T
            xb = x_scr[t0:t0 + RB, :]
            xf = xb.astype(F32)
            m = jnp.mean(xf, axis=-1, keepdims=True)
            xc = xf - m
            r = jax.lax.rsqrt(jnp.mean(xc * xc, axis=-1, keepdims=True) + _EPS)
            xn_scr[t0 // BQ, t0 % BQ:t0 % BQ + RB, :] = (xc * r).astype(BF16)
            kf = (_dot(xb, wqkv_scr[1]) - m * wk_cs) * r
            for g in range(NG):
                k_scr[g, t0 // 2:(t0 + RB) // 2, :] = _pack(kf[:, g * 128:(g + 1) * 128])
                for c in range(NC):
                    lo, hi = c * CK + MK - t0, (c + 1) * CK - t0
                    if lo >= 0 and hi <= RB:
                        kf_scr[g, c] = kf[lo:hi, g * 128:(g + 1) * 128].astype(BF16).astype(F32)
            kk = jnp.max((kf * kf).reshape(RB // 64, 64, D), axis=0)
            kk_max = kk if kk_max is None else jnp.maximum(kk_max, kk)

        def kn_bound():
            seg = (jax.lax.broadcasted_iota(jnp.int32, (D, 128), 0) // Dh
                   == jax.lax.broadcasted_iota(jnp.int32, (D, 128), 1)).astype(BF16)
            return jnp.max(_dot(jnp.minimum(kk_max * 1.03, _BIG).astype(BF16), seg))

        qscale = (Dh ** -0.5) * _LOG2E

        def proj(tb, carry):
            qn_max, v_max = carry
            qv = _dot_nt(wt_scr[...], xn_scr[tb])
            qf = (qv[0:D] * qscale).astype(BF16).astype(F32)
            qt_scr[tb] = _pack(qf).reshape(H, Dh // 2, BQ)
            qf_scr[tb] = qf.reshape(H, Dh, BQ)
            qg_scr[tb] = qf.reshape(H, Dh, BQ)[:, 0:8, :]
            for cc in range(CPB):
                vt_scr[tb * CPB + cc] = _pack(qv[D:2 * D, cc * CK:(cc + 1) * CK]).reshape(H, Dh // 2, CK)
            qn_max = jnp.maximum(qn_max, _fold_max(jnp.sum((qf * qf).reshape(H, Dh, BQ), axis=1)))
            v_max = jnp.maximum(v_max, _fold_max(jnp.abs(qv[D:2 * D])))
            wot_scr[tb] = wo_scr[tb * 128:(tb + 1) * 128, :].T
            for hh in range(tb * HG // NQ, (tb + 1) * HG // NQ):
                grps = [(2 * hh + 1, 1), (2 * hh, 0) if hh else (NGRP, CB)]
                kv = jnp.concatenate([kf_scr[0, c] for _, c in grps], axis=0)
                for d in range(Dh):
                    lane = hh * Dh + d
                    v = jnp.broadcast_to(kv[:, lane:lane + 1], (2 * VK, 128))
                    for n, (grp, _) in enumerate(grps):
                        kb_scr[0, grp - 1, d] = v[n * VK:(n + 1) * VK]
            return qn_max, v_max

        qn_max, v_max = jnp.zeros((8, 128), F32), jnp.zeros((8, 128), F32)
        for tb in range(NQ):
            qn_max, v_max = proj(tb, (qn_max, v_max))
            if tb == NQ - 2:
                kn_max = kn_bound()
        for tb in range(NQ):
            wq0 = jnp.concatenate([_unpack(qt_scr[tb, 0]), jnp.zeros((128 - Dh, BQ), BF16)], axis=0)
            sv_scr[tb] = _dot(_unpack(k_scr[0, MK // 2:CK // 2, :]), wq0)
        bound2 = jnp.max(qn_max) * kn_max
        fast = jnp.logical_and(jnp.logical_and(bound2 <= _SAFE_LOG2 * _SAFE_LOG2, kn_max < 0.5 * _BIG),
                               jnp.max(v_max) <= _SAFE_V)

        def pv_carry(t):
            h = (t // NCB) * HG + HG - 1
            c = (t % NCB) * CB + CB - 1
            o = _dot(_unpack(vt_scr[c, h]), pc_scr[...])
            acc_scr[NQ - 1, h, 0:Dh, :] = o + acc_scr[NQ - 1, h, 0:Dh, :]

        @pl.when(fast)
        def _fast():
            def body(it, carry):
                its = [it, jnp.minimum(it + 1, NIT - 1), jnp.minimum(it + 2, NIT - 1)]
                gs = [t // NCB for t in its]
                cs = [(t % NCB) * CB for t in its]
                g, c0 = gs[0], cs[0]
                seq = [(hh, cc, qb) for hh in range(HG) for cc in range(CB) for qb in range(NQ)]
                state = dict(tok=None, xtok=None)
                sv, pts, part, lsum = {}, {}, {}, {}

                def group(grp):
                    b, r = grp // NGRP, grp % NGRP
                    return gs[b], cs[b] + r % CB, r // CB

                def vpu(j):
                    grp, qb = j // NQ, j % NQ
                    gg, _, hh = group(grp)

                    def side(idx):
                        if idx % 2:
                            return
                        d = idx // 2
                        gb, cb, hb = group(grp + NGRP)
                        lane = hb * Dh + d
                        kv = kf_scr[gb, cb]
                        if d in _XL and state['xtok'] is not None:
                            kv = jnp.concatenate([kv[0:8] + state['xtok'], kv[8:]], axis=0)
                        v = jnp.broadcast_to(kv[:, lane:lane + 1], (VK, 128))
                        kb_scr[it + 1, grp - 1, d] = v
                        if d in _XL:
                            w = v[0:8]
                            state['xtok'] = w - w
                    r = vpu_scores(lambda d, r: kb_scr[it, grp - 1, d, r:r + 16, :],
                                   gg * HG + hh, qb, state, side)
                    if j >= NSTEP:
                        sv_scr[j - NSTEP] = r
                    else:
                        sv[j] = r

                def qk(j):
                    hh, cc, qb = seq[j]
                    parts = []
                    if hh > 0:
                        parts.append(jnp.zeros((hh * Dh, BQ), BF16))
                    parts.append(_unpack(qt_scr[qb, g * HG + hh]))
                    if hh < HG - 1:
                        parts.append(jnp.zeros(((HG - 1 - hh) * Dh, BQ), BF16))
                    wq = jnp.concatenate(parts, axis=0)
                    r0 = pl.multiple_of((c0 + cc) * (CK // 2), CK // 2)
                    r = sv_scr[j] if j < A else sv.pop(j)
                    st = _dot(_unpack(k_scr[g, pl.ds(r0, MK // 2), :]), wq)
                    p = jnp.exp2(jnp.concatenate([st, r], axis=0))
                    ps = jnp.sum(p.reshape(CK // 8, 8, BQ), axis=0)
                    lsum[(hh, qb)] = ps if cc == 0 else ps + lsum[(hh, qb)]
                    pts[j] = p

                def pv(j):
                    hh, cc, qb = seq[j]
                    h = g * HG + hh
                    last = (hh, qb) == (HG - 1, NQ - 1)
                    o = _dot(_unpack(vt_scr[c0 + cc, h]), pts.pop(j))
                    if cc == 0:
                        part[(hh, qb)] = o + acc_scr[qb, h, 0:Dh, :]
                    else:
                        part[(hh, qb)] = o + part[(hh, qb)]
                    if cc == CB - 1 - (1 if last else 0):
                        acc_scr[qb, h, 0:Dh, :] = part.pop((hh, qb))
                    if cc == CB - 1:
                        acc_scr[qb, h, Dh:Dh + 8, :] = lsum.pop((hh, qb)) + acc_scr[qb, h, Dh:Dh + 8, :]

                for j in range(NSTEP + 1):
                    if j < NSTEP:
                        qk(j)
                        vpu(j + A)
                    if j == 0:
                        pv_carry(jnp.maximum(it - 1, 0))
                    elif j == NSTEP:
                        pc_scr[...] = pts.pop(j - 1)
                        h = g * HG + HG - 1
                        acc_scr[NQ - 1, h, Dh:Dh + 8, :] = (lsum.pop((HG - 1, NQ - 1))
                                                            + acc_scr[NQ - 1, h, Dh:Dh + 8, :])
                    else:
                        pv(j - 1)
                return carry
            jax.lax.fori_loop(0, NIT, body, 0)
            pv_carry(NIT - 1)
            v = kb_scr[NIT, 0, 0, 0:8, :]
            acc_scr[0, 0, Dh:Dh + 8, 0:128] = acc_scr[0, 0, Dh:Dh + 8, 0:128] + (v - v)

        @pl.when(jnp.logical_not(fast))
        def _slow():
            def head(h, carry):
                g = h // HG
                wq_scr[...] = jnp.zeros(wq_scr.shape, U32)
                r0 = pl.multiple_of((h % HG) * (Dh // 2), Dh // 2)
                for qb in range(NQ):
                    wq_scr[pl.ds(r0, Dh // 2), qb * BQ:(qb + 1) * BQ] = qt_scr[qb, h]

                def scores(c):
                    kc = k_scr[g, pl.ds(pl.multiple_of(c * (CK // 2), CK // 2), CK // 2), :]
                    return _dot(_unpack(kc), _unpack(wq_scr[...]))

                def mx(c, m):
                    return jnp.maximum(m, jnp.max(scores(c).reshape(CK // 8, 8, S), axis=0))
                m8 = jax.lax.fori_loop(0, NC, mx, jnp.full((8, S), -jnp.inf, F32))
                m = jnp.max(m8, axis=0, keepdims=True)

                def acc(c, carry):
                    o, l = carry
                    p = jnp.exp2(scores(c) - m)
                    return (o + _dot(_unpack(vt_scr[c, h]), p.astype(BF16)),
                            l + jnp.sum(p.reshape(CK // 8, 8, S), axis=0))
                o, l = jax.lax.fori_loop(0, NC, acc, (jnp.zeros((Dh, S), F32), jnp.zeros((8, S), F32)))
                for qb in range(NQ):
                    acc_scr[qb, h, 0:Dh, :] = o[:, qb * BQ:(qb + 1) * BQ]
                    acc_scr[qb, h, Dh:Dh + 8, :] = l[:, qb * BQ:(qb + 1) * BQ]
                return carry
            jax.lax.fori_loop(0, H, head, 0)

        for cp in late_copies[1:]:
            cp.wait()

    a = acc_scr[i]
    l = jnp.sum(a[:, Dh:Dh + 8, :], axis=1, keepdims=True)
    inv = pl.reciprocal(l, approx=True)
    inv = inv * (2.0 - l * inv)
    ot = (a[:, 0:Dh, :] * inv).reshape(D, BQ)
    b1 = b1_scr[...].astype(F32)[None, :]
    b2 = b2_scr[...].astype(F32)[None, :]
    r0 = pl.multiple_of(i * BQ, BQ)
    ao = _dot(jnp.concatenate([wot_scr[t] for t in range(NQ)], axis=1), ot).T
    h = x_scr[pl.ds(r0, BQ), :].astype(F32) + ao
    hc = h - jnp.mean(h, axis=-1, keepdims=True)
    r = jax.lax.rsqrt(jnp.mean(hc * hc, axis=-1, keepdims=True) + _EPS)
    z = _dot(hc.astype(BF16), w1_scr[...]) * r + b1
    gl = jax.nn.gelu(z, approximate=True).astype(BF16)
    y = _dot(gl, w2_scr[...]) + b2
    o_ref[...] = (h + y).astype(o_ref.dtype)


@jax.jit
def pallas_sequential_preLN__softmax_full_mha__dense_activation_gelu__prompt_kernel(
    A_x: jax.Array,
    A_wqkv: jax.Array,
    A_wo: jax.Array,
    B_x: jax.Array,
    B_w1: jax.Array,
    B_b1: jax.Array,
    B_w2: jax.Array,
    B_b2: jax.Array,
):
    del B_x
    B, S, D = A_x.shape
    assert B == 1 and S == _XB[-1]
    F = B_w1.shape[1]
    H, BQ, CK, VK = _H, _BQ, _CK, _VK
    Dh = D // H
    NQ = S // BQ
    NC = S // CK
    NIT = (D // 128) * (NC // _CB)
    NGRP = (128 // Dh) * _CB

    out = pl.pallas_call(
        functools.partial(_kernel, S=S, D=D),
        grid=(NQ,),
        in_specs=[pl.BlockSpec(memory_space=pl.ANY)] * 7,
        out_specs=pl.BlockSpec((BQ, D), lambda i: (i, 0)),
        out_shape=jax.ShapeDtypeStruct((S, D), A_x.dtype),
        scratch_shapes=[
            pltpu.VMEM((S, D), BF16),
            pltpu.VMEM((NQ, BQ, D), BF16),
            pltpu.VMEM((3, D, D), BF16),
            pltpu.VMEM((D, D), BF16),
            pltpu.VMEM((D, F), BF16),
            pltpu.VMEM((F, D), BF16),
            pltpu.VMEM((2 * D, D), BF16),
            pltpu.VMEM((D // 128, S // 2, 128), U32),
            pltpu.VMEM((D // 128, NC, VK, 128), F32),
            pltpu.VMEM((NQ, H, Dh // 2, BQ), U32),
            pltpu.VMEM((NQ, H, Dh, BQ), F32),
            pltpu.VMEM((NC, H, Dh // 2, CK), U32),
            pltpu.VMEM((NQ, H, Dh + 8, BQ), F32),
            pltpu.VMEM((NIT + 1, NGRP, Dh, VK, 128), F32),
            pltpu.VMEM((NQ, VK, BQ), F32),
            pltpu.VMEM((64, S), U32),
            pltpu.VMEM((F,), BF16),
            pltpu.VMEM((D,), BF16),
            pltpu.VMEM((CK, BQ), F32),
            pltpu.VMEM((NQ, H, 8, BQ), F32),
            pltpu.VMEM((NQ, D, 128), BF16),
            pltpu.SemaphoreType.DMA((8 + len(_XB) - 1,)),
        ],
        compiler_params=pltpu.CompilerParams(
            dimension_semantics=("arbitrary",),
            vmem_limit_bytes=120 * 1024 * 1024),
    )(A_x.reshape(S, D), A_wqkv, A_wo, B_w1, B_b1, B_w2, B_b2)
    return out.reshape(B, S, D)
```
